```python
import os as _os
_os.environ.setdefault("JAX_PLATFORMS", "cpu")
import jax
import jax.numpy as jnp

def _softmax(x, axis=-1):
    return jax.nn.softmax(x, axis=axis)
def _gelu(x):
    return jax.nn.gelu(x, approximate=True)
def _silu(x):
    return jax.nn.silu(x)
def _sigmoid(x):
    return jax.nn.sigmoid(x)
def _layernorm(x, axis=-1, eps=1e-5):
    m = jnp.mean(x, axis=axis, keepdims=True)
    v = jnp.var(x, axis=axis, keepdims=True)
    return (x - m) / jnp.sqrt(v + eps)
def _scatter_add(tgt, idx, src, axis=0):
    return tgt.at[idx].add(src)
def _segment_sum(src, seg, n):
    return jax.ops.segment_sum(src, seg, n)
class _Rng:
    def __init__(self, key):
        self._k = key
    def _next(self):
        self._k, sub = jax.random.split(self._k)
        return sub
    def normal(self, shape):
        return jax.random.normal(self._next(), shape, dtype=jnp.bfloat16)
    def randint(self, lo, hi, shape):
        return jax.random.randint(self._next(), shape, lo, hi, dtype=jnp.int32)
    def uniform(self, shape, lo=0.0, hi=1.0):
        return jax.random.uniform(self._next(), shape, jnp.bfloat16, lo, hi)
    def permutation(self, n):
        return jax.random.permutation(self._next(), n)


kernel_name = 'interleave_layers__spectral_gfnet__dense_activation_gelu__prompt'

def setup_inputs():
    _rng = _Rng(jax.random.key(int.from_bytes(__import__("os").urandom(4), "little")))
    _w = (lambda a: (lambda t: t.astype(jnp.bfloat16) if jnp.issubdtype(t.dtype, jnp.floating) else t)(jnp.asarray(a)))
    def _A_setup():
        B, S, D = 1, 2048, 640
        Df = D // 2 + 1
        return {
            "x": _w((lambda *s: _rng.normal(s) * 0.05)(B, S, D)),
            "w_r": _w((lambda *s: _rng.normal(s) * 0.2)(S, Df) * 0.02),
            "w_i": _w((lambda *s: _rng.normal(s) * 0.2)(S, Df) * 0.02),
        }
    _A_in = _A_setup()

    def _B_setup():
        B, S, D, F = 1, 2048, 640, 1728
        return {
            "x": _w((lambda *s: _rng.normal(s) * 0.05)(B, S, D)),
            "w1": _w((lambda *s: _rng.normal(s) * 0.1)(D, F) * (D ** -0.5)),
            "b1": _w((lambda *s: _rng.normal(s) * 0.1)(F) * 0.01),
            "w2": _w((lambda *s: _rng.normal(s) * 0.1)(F, D) * (F ** -0.5)),
            "b2": _w((lambda *s: _rng.normal(s) * 0.1)(D) * 0.01),
        }
    _B_in = _B_setup()

    return {
        "A_x": _A_in["x"],
        "A_w_r": _A_in["w_r"],
        "A_w_i": _A_in["w_i"],
        "B_x": _B_in["x"],
        "B_w1": _B_in["w1"],
        "B_b1": _B_in["b1"],
        "B_w2": _B_in["w2"],
        "B_b2": _B_in["b2"],
    }

def reference(A_x, A_w_r, A_w_i, B_x, B_w1, B_b1, B_w2, B_b2):
    def _A_ref(x, w_r, w_i):
        B, S, D = x.shape
        X = (lambda x, axes=(-2,-1): jnp.fft.rfft2(x.astype(jnp.float32), axes=axes))(x, axes=(-2, -1))
        W = w_r + 1j * w_i
        X = X * W
        y = (lambda x, s, axes=(-2,-1): jnp.fft.irfft2(x, s=s, axes=axes).astype(jnp.bfloat16))(X, (S, D), axes=(-2, -1))
        return y

    def _B_ref(x, w1, b1, w2, b2):
        h = jnp.einsum("bsd,df->bsf", x, w1) + b1
        h = _gelu(h)
        return jnp.einsum("bsf,fd->bsd", h, w2) + b2

    x = A_x
    x = x + _A_ref(_layernorm(x, axis=-1), A_w_r, A_w_i)
    x = x + _B_ref(_layernorm(x, axis=-1), B_w1, B_b1, B_w2, B_b2)
    x = x + _A_ref(_layernorm(x, axis=-1), A_w_r, A_w_i)
    x = x + _B_ref(_layernorm(x, axis=-1), B_w1, B_b1, B_w2, B_b2)
    return x
```

```python
import functools
import numpy as np
import jax, jax.numpy as jnp
from jax import lax
from jax.experimental import pallas as pl
from jax.experimental.pallas import tpu as pltpu
import ml_dtypes

S, D, F = 2048, 640, 1728
BF = ml_dtypes.bfloat16

def _lcols():
    e = np.arange(128)
    lA = np.where(e < 64, 1 + 5 * e, 4 + 5 * (e - 64))
    lB = np.where(e < 64, 2 + 5 * e, 3 + 5 * (e - 64))
    l0 = np.where(e <= 64, 5 * e, -1)
    return lA, lB, l0

def _consts():
    lA, lB, l0 = _lcols()
    q = np.arange(128)
    sgn = np.where(np.arange(128) < 64, 1.0, -1.0)
    def MN(l):
        ph = 2 * np.pi * ((q[:, None] * l[None, :]) % D) / D
        c, s = np.cos(ph), np.sin(ph)
        M = np.block([[c, -s], [sgn * s, sgn * c]])
        N = 2.0 / (S * D) * np.block([[c.T, sgn[:, None] * s.T], [-s.T, sgn[:, None] * c.T]])
        return M, N
    MA, NA = MN(lA); MB, NB = MN(lB)
    v = (l0 >= 0)
    ph = 2 * np.pi * ((q[:, None] * np.maximum(l0, 0)[None, :]) % D) / D
    c, s = np.cos(ph) * v, np.sin(ph) * v
    s = np.where(np.abs(s) < 1e-9, 0.0, s)
    M0 = np.concatenate([c, -s], axis=1)
    cl = np.where((l0 == 0) | (l0 == D // 2), 1.0, 2.0) * v / (S * D)
    N0 = np.concatenate([c.T * cl[:, None], -s.T * cl[:, None]], axis=0)
    d = np.arange(128); b = np.arange(128)
    rho = np.arange(256)
    src = ((rho // 8) % 2) * 128 + (rho // 16) * 8 + rho % 8
    CSF = np.zeros((16, 256, 256)); CST = np.zeros((16, 256, 256))
    for cc in range(16):
        ph = 2 * np.pi * ((b[None, :] * (cc + 16 * d[:, None])) % S) / S
        C, Sn = np.cos(ph), np.sin(ph)
        CSF[cc] = np.block([[C, Sn], [-Sn, C]])[:, src]
        CST[cc] = np.block([[C.T, -Sn.T], [Sn.T, C.T]])
    lall = np.concatenate([lA, lB, l0])
    PC = np.zeros((D // 2 + 1, 384))
    for n, l in enumerate(lall):
        if l >= 0:
            PC[l, n] = 1.0
    P1 = np.zeros((128, 128))
    for c in range(16):
        for j in range(8):
            P1[8 * c + j, 16 * j + c] = 1.0
    MF = np.concatenate([MA, MB], axis=0)
    MFZ = np.concatenate([MF, np.concatenate([M0, M0 * 0], 0)], axis=0)
    NI = np.concatenate([NA, NB, np.concatenate([N0, N0 * 0], 1)], axis=0)
    out = dict(MFZ=MFZ, NI=NI, CSF=CSF, CST=CST, PC=PC, P1=P1)
    return {k: v.astype(np.float32).astype(BF) for k, v in out.items()}

_K = _consts()

C16 = [np.cos(2 * np.pi * k / 16) for k in range(16)]
S16 = [np.sin(2 * np.pi * k / 16) for k in range(16)]

def _cmul_w16(re, im, k, sign):
    k = k % 16
    if sign < 0:
        k = (16 - k) % 16
    if k == 0: return re, im
    if k == 4: return -im, re
    if k == 8: return -re, -im
    if k == 12: return im, -re
    c, s = float(C16[k]), float(S16[k])
    if k % 2 == 0:
        r = abs(c)
        sc, ss = (c > 0), (s > 0)
        a = (re if sc else -re)
        return None
    return re * c - im * s, re * s + im * c

def _tw(re, im, k, sign):
    k = k % 16
    kk = k if sign > 0 else (16 - k) % 16
    if kk == 0: return re, im
    if kk == 4: return -im, re
    if kk == 8: return -re, -im
    if kk == 12: return im, -re
    c, s = float(C16[kk]), float(S16[kk])
    if kk % 2 == 0:
        r = float(np.sqrt(0.5))
        if kk == 2:   return (re - im) * r, (re + im) * r
        if kk == 6:   return (re + im) * (-r), (re - im) * r
        if kk == 10:  return (im - re) * r, (re + im) * (-r)
        if kk == 14:  return (re + im) * r, (im - re) * r
    return re * c - im * s, re * s + im * c

def _dft4(x, sign):
    (a_r, a_i), (b_r, b_i), (c_r, c_i), (d_r, d_i) = x
    s0r, s0i = a_r + c_r, a_i + c_i
    s1r, s1i = a_r - c_r, a_i - c_i
    s2r, s2i = b_r + d_r, b_i + d_i
    s3r, s3i = b_r - d_r, b_i - d_i
    X0 = (s0r + s2r, s0i + s2i)
    X2 = (s0r - s2r, s0i - s2i)
    if sign < 0:
        X1 = (s1r + s3i, s1i - s3r)
        X3 = (s1r - s3i, s1i + s3r)
    else:
        X1 = (s1r - s3i, s1i + s3r)
        X3 = (s1r + s3i, s1i - s3r)
    return [X0, X1, X2, X3]

def _fft16(x, sign):
    inner = []
    for n1 in range(4):
        y = _dft4([x[n1 + 4 * n2] for n2 in range(4)], sign)
        inner.append([_tw(y[k2][0], y[k2][1], n1 * k2, sign) for k2 in range(4)])
    out = [None] * 16
    for k2 in range(4):
        z = _dft4([inner[n1][k2] for n1 in range(4)], sign)
        for k1 in range(4):
            out[k2 + 4 * k1] = z[k1]
    return out

C5_1, C5_2 = float(np.cos(2 * np.pi / 5)), float(np.cos(4 * np.pi / 5))
S5_1, S5_2 = float(np.sin(2 * np.pi / 5)), float(np.sin(4 * np.pi / 5))

def _ln(x):
    m = jnp.mean(x, axis=-1, keepdims=True)
    xc = x - m
    v = jnp.mean(xc * xc, axis=-1, keepdims=True)
    return xc * lax.rsqrt(v + 1e-5)

def _gelu(h):
    c0 = 0.7978845608028654
    return 0.5 * h * (1.0 + jnp.tanh(c0 * (h + 0.044715 * h * h * h)))

def _radix5_fwd(xn):
    x0, x1, x2, x3, x4 = [xn[:, 128 * p:128 * (p + 1)] for p in range(5)]
    t1, t2, t3, t4 = x1 + x4, x2 + x3, x1 - x4, x2 - x3
    z0 = x0 + t1 + t2
    z1r = x0 + C5_1 * t1 + C5_2 * t2
    z2r = x0 + C5_2 * t1 + C5_1 * t2
    z1i = -(S5_1 * t3 + S5_2 * t4)
    z2i = -(S5_2 * t3 - S5_1 * t4)
    return z0, z1r, z1i, z2r, z2i

def _radix5_inv(T0, T1r, T1i, T2r, T2i):
    y0 = T0 + T1r + T2r
    E1 = T0 + C5_1 * T1r + C5_2 * T2r
    E2 = T0 + C5_2 * T1r + C5_1 * T2r
    O1 = S5_1 * T1i + S5_2 * T2i
    O2 = S5_2 * T1i - S5_1 * T2i
    return y0, E1 - O1, E2 - O2, E2 + O2, E1 + O1

def make_kernel(R=32, phases="all"):
    G = R // 8
    NCH = 128 // R
    M = 128 * G
    f32, bf16 = jnp.float32, jnp.bfloat16

    def kernel(x_hbm, wr_hbm, wi_hbm, w1_hbm, b1_hbm, w2_hbm, b2_hbm,
               mfz_hbm, ni_hbm, csf_hbm, cst_hbm, pc_hbm, p1_hbm,
               o_hbm,
               xst, wr_v, wi_v, w1_v, b1_v, w2_v, b2_v, mfz_v, ni_v, csf_v, cst_v, pc_v, p1_v,
               xs, ybuf, bbuf, wc, ost, sems, osem):
        xcopies = [pltpu.make_async_copy(x_hbm.at[:, j], xst.at[j], sems.at[j]) for j in range(NCH)]
        others = [(mfz_hbm, mfz_v), (pc_hbm, pc_v), (p1_hbm, p1_v), (wr_hbm, wr_v), (wi_hbm, wi_v),
                  (csf_hbm, csf_v), (cst_hbm, cst_v), (ni_hbm, ni_v), (w1_hbm, w1_v), (b1_hbm, b1_v),
                  (w2_hbm, w2_v), (b2_hbm, b2_v)]
        ocopies = [pltpu.make_async_copy(s, d, sems.at[NCH + i]) for i, (s, d) in enumerate(others)]
        for cp in xcopies: cp.start()
        for cp in ocopies: cp.start()
        cp_mfz, cp_pc, cp_p1, cp_wr, cp_wi, cp_csf, cp_cst, cp_ni, cp_w1, cp_b1, cp_w2, cp_b2 = ocopies

        def head(xv, j):
            xn = _ln(xv)
            z0, z1r, z1i, z2r, z2i = _radix5_fwd(xn)
            za = jnp.concatenate([z1r, z1i], axis=1).astype(bf16)
            zb = jnp.concatenate([z2r, z2i], axis=1).astype(bf16)
            zz = z0.astype(bf16)
            U = [jnp.dot(za, mfz_v[0:256, :], preferred_element_type=f32),
                 jnp.dot(zb, mfz_v[256:512, :], preferred_element_type=f32),
                 jnp.dot(zz, mfz_v[512:640, :], preferred_element_type=f32)]
            for g in range(G):
                gp = j * G + g
                row0 = 16 * gp if isinstance(gp, int) else pl.multiple_of(16 * gp, 16)
                for t in range(3):
                    ins = [(U[t][128 * g + 8 * a:128 * g + 8 * a + 8, 0:128],
                            U[t][128 * g + 8 * a:128 * g + 8 * a + 8, 128:256]) for a in range(16)]
                    outs = _fft16(ins, -1)
                    for c in range(16):
                        v = jnp.concatenate([outs[c][0], outs[c][1]], axis=0).astype(bf16)
                        ybuf[c, pl.ds(row0, 16), 128 * t:128 * (t + 1)] = v

        def sphase():
            def body(c, _):
                Y = ybuf[c]
                X = jnp.dot(csf_v[c], Y, preferred_element_type=f32)
                Xr, Xi = X[0:128], X[128:256]
                Wr, Wi = wc[c, 0:128, :], wc[c, 128:256, :]
                Zr = Xr * Wr - Xi * Wi
                Zi = Xr * Wi + Xi * Wr
                Z = jnp.concatenate([Zr, Zi], axis=0).astype(bf16)
                bbuf[c] = jnp.dot(cst_v[c], Z, preferred_element_type=f32)
                return 0
            lax.fori_loop(0, 16, body, 0)

        def tail(j):
            A = [[], [], []]
            for g in range(G):
                gp = j * G + g
                r0 = pl.multiple_of(8 * gp, 8)
                for t in range(3):
                    ins = [(bbuf[c, pl.ds(r0, 8), 128 * t:128 * (t + 1)],
                            bbuf[c, pl.ds(128 + r0, 8), 128 * t:128 * (t + 1)]) for c in range(16)]
                    outs = _fft16(ins, +1)
                    ar = jnp.concatenate([o[0] for o in outs], axis=0)
                    ai = jnp.concatenate([o[1] for o in outs], axis=0)
                    A[t].append(jnp.concatenate([ar, ai], axis=1).astype(bf16))
            A = [jnp.concatenate(a, axis=0) if len(a) > 1 else a[0] for a in A]
            TA = jnp.dot(A[0], ni_v[0:256, :], preferred_element_type=f32)
            TB = jnp.dot(A[1], ni_v[256:512, :], preferred_element_type=f32)
            T0 = jnp.dot(A[2], ni_v[512:768, 0:128], preferred_element_type=f32)
            ys = _radix5_inv(T0, TA[:, 0:128], TA[:, 128:256], TB[:, 0:128], TB[:, 128:256])
            return jnp.concatenate(ys, axis=1)

        def mlp(x):
            xn = _ln(x).astype(bf16)
            h = lax.dot_general(xn, w1_v[...], (((1,), (1,)), ((), ())), preferred_element_type=f32) + b1_v[...].astype(f32).reshape(1, F)
            g = _gelu(h).astype(bf16)
            return x + jnp.dot(g, w2_v[...], preferred_element_type=f32) + b2_v[...].astype(f32).reshape(1, D)

        cp_mfz.wait()
        def head0(j, _):
            pltpu.make_async_copy(x_hbm.at[:, 0], xst.at[j], sems.at[j]).wait()
            v = xst[j].astype(f32)
            xv = jnp.concatenate([v[:, 8 * g:8 * g + 8, :].reshape(128, D) for g in range(G)], axis=0)
            r0 = pl.multiple_of(j * M, M)
            xs[pl.ds(r0, M), :] = xv
            head(xv, j)
            return 0
        lax.fori_loop(0, NCH, head0, 0)

        cp_pc.wait(); cp_p1.wait(); cp_wr.wait(); cp_wi.wait()
        def wprep(m, _):
            r0 = pl.multiple_of(m * 128, 128)
            d0 = pl.multiple_of(m * 8, 8)
            for h, wv in enumerate((wr_v, wi_v)):
                T = lax.dot_general(p1_v[...], wv[:, pl.ds(r0, 128)], (((1,), (1,)), ((), ())), preferred_element_type=f32).astype(bf16)
                T = jnp.dot(T, pc_v[...], preferred_element_type=f32)
                for c in range(16):
                    wc[c, pl.ds(128 * h + d0, 8), :] = T[8 * c:8 * c + 8, :]
            return 0
        lax.fori_loop(0, 16, wprep, 0)

        cp_csf.wait(); cp_cst.wait()
        sphase()
        cp_ni.wait(); cp_w1.wait(); cp_b1.wait(); cp_w2.wait(); cp_b2.wait()

        def mid(j, _):
            r0 = pl.multiple_of(j * M, M)
            x = xs[pl.ds(r0, M), :] + tail(j)
            x = mlp(x)
            xs[pl.ds(r0, M), :] = x
            head(x, j)
            return 0
        lax.fori_loop(0, NCH, mid, 0)
        sphase()

        def last(j, _):
            r0 = pl.multiple_of(j * M, M)
            x = xs[pl.ds(r0, M), :] + tail(j)
            x = mlp(x)
            for a in range(16):
                v = jnp.concatenate([x[128 * g + 8 * a:128 * g + 8 * a + 8, :] for g in range(G)], axis=0)
                ost[j, a] = v.astype(bf16)
            pltpu.make_async_copy(ost.at[j], o_hbm.at[:, j], osem.at[j]).start()
            return 0
        lax.fori_loop(0, NCH, last, 0)
        for j in range(NCH):
            pltpu.make_async_copy(ost.at[j], o_hbm.at[:, j], osem.at[j]).wait()

    def fn(A_x, A_w_r, A_w_i, B_x, B_w1, B_b1, B_w2, B_b2):
        x4 = A_x.reshape(16, NCH, R, D)
        any_spec = pl.BlockSpec(memory_space=pltpu.HBM)
        scratch = [
            pltpu.VMEM((NCH, 16, R, D), bf16), pltpu.VMEM((D // 2 + 1, S), bf16), pltpu.VMEM((D // 2 + 1, S), bf16),
            pltpu.VMEM((F, D), bf16), pltpu.VMEM((F,), bf16), pltpu.VMEM((F, D), bf16), pltpu.VMEM((D,), bf16),
            pltpu.VMEM((768, 256), bf16), pltpu.VMEM((768, 256), bf16),
            pltpu.VMEM((16, 256, 256), bf16), pltpu.VMEM((16, 256, 256), bf16),
            pltpu.VMEM((D // 2 + 1, 384), bf16), pltpu.VMEM((128, 128), bf16),
            pltpu.VMEM((S, D), f32), pltpu.VMEM((16, 256, 384), bf16), pltpu.VMEM((16, 256, 384), f32),
            pltpu.VMEM((16, 256, 384), f32), pltpu.VMEM((NCH, 16, R, D), bf16),
            pltpu.SemaphoreType.DMA((NCH + 12,)), pltpu.SemaphoreType.DMA((NCH,)),
        ]
        K = _K
        out = pl.pallas_call(
            kernel,
            out_shape=jax.ShapeDtypeStruct((16, NCH, R, D), bf16),
            in_specs=[any_spec] * 13,
            out_specs=any_spec,
            scratch_shapes=scratch,
            compiler_params=pltpu.CompilerParams(vmem_limit_bytes=110 * 1024 * 1024),
        )(x4, A_w_r.T, A_w_i.T, B_w1.T, B_b1, B_w2, B_b2,
          K["MFZ"], K["NI"], K["CSF"], K["CST"], K["PC"], K["P1"])
        return out.reshape(1, S, D)
    return fn


_FN = make_kernel(**dict(R=32))


@jax.jit
def pallas_interleave_layers__spectral_gfnet__dense_activation_gelu__prompt_kernel(
    A_x: jax.Array,
    A_w_r: jax.Array,
    A_w_i: jax.Array,
    B_x: jax.Array,
    B_w1: jax.Array,
    B_b1: jax.Array,
    B_w2: jax.Array,
    B_b2: jax.Array,
):
    return _FN(A_x, A_w_r, A_w_i, B_x, B_w1, B_b1, B_w2, B_b2)
```

```python
import numpy as np
import jax, jax.numpy as jnp
from jax import lax
from jax.experimental import pallas as pl
from jax.experimental.pallas import tpu as pltpu
import ml_dtypes

S, D, F = 2048, 640, 1728
DF = D // 2 + 1
BF = ml_dtypes.bfloat16

def _tiles(m):
    r, c = m.shape
    return np.ascontiguousarray(m.reshape(r, c // 128, 128).transpose(1, 0, 2))

def _consts():
    e = np.arange(128)
    lA = np.where(e < 64, 1 + 5 * e, 4 + 5 * (e - 64))
    lB = np.where(e < 64, 2 + 5 * e, 3 + 5 * (e - 64))
    q = np.arange(128)
    sgn = np.where(e < 64, 1.0, -1.0)
    def MN(l):
        ph = 2 * np.pi * ((q[:, None] * l[None, :]) % D) / D
        c, s = np.cos(ph), np.sin(ph)
        M = np.block([[c, -s], [sgn * s, sgn * c]])
        N = 2.0 / (S * D) * np.block([[c.T, sgn[:, None] * s.T], [-s.T, sgn[:, None] * c.T]])
        return M, N
    MA, NA = MN(lA); MB, NB = MN(lB)
    e0 = np.arange(64)
    l0 = np.where(e0 == 0, D // 2, 5 * e0)
    ph = 2 * np.pi * ((q[:, None] * l0[None, :]) % D) / D
    c, s = np.cos(ph), np.sin(ph)
    s = np.where(np.abs(s) < 1e-9, 0.0, s)
    M0 = np.concatenate([c, -s], axis=1)
    cl = np.where(e0 == 0, 1.0, 2.0) / (S * D)
    N0 = np.concatenate([c.T * cl[:, None], -s.T * cl[:, None]], axis=0)
    d = np.arange(128); b = np.arange(128)
    CSF = np.zeros((16, 256, 128)); CST = np.zeros((16, 256, 128))
    CSF3 = np.zeros((16, 384, 128)); CST3 = np.zeros((16, 384, 128))
    for cc in range(16):
        ph = 2 * np.pi * ((b[None, :] * (cc + 16 * d[:, None])) % S) / S
        C, Sn = np.cos(ph), np.sin(ph)
        CSF[cc] = np.concatenate([C, Sn], axis=0)
        CST[cc] = np.concatenate([C.T, Sn.T], axis=0)
        CSF3[cc] = np.concatenate([C, C - Sn, C + Sn], axis=0)
        CST3[cc] = np.concatenate([C.T, C.T + Sn.T, C.T - Sn.T], axis=0)
    P1 = np.zeros((128, 128))
    for cc in range(16):
        for j in range(8):
            P1[8 * cc + j, 16 * j + cc] = 1.0
    s1 = np.sin(2 * np.pi / 5)
    MA = MA.copy(); MB = MB.copy(); NA = NA.copy(); NB = NB.copy()
    MA[128:] *= -s1
    MB[128:] *= -s1
    NA[:, 128:] *= s1
    NB[:, 128:] *= s1
    def MN3(l, zi_scale):
        ph = 2 * np.pi * ((q[:, None] * l[None, :]) % D) / D
        c, s = np.cos(ph), sgn[None, :] * np.sin(ph)
        F3 = np.stack([c, zi_scale * (c - s), c + s])
        I3 = 2.0 / (S * D) * np.stack([c.T, (c + s).T, (s - c).T])
        return F3, I3
    F3A, I3A = MN3(lA, -s1); F3B, I3B = MN3(lB, -s1)
    MF3 = np.concatenate([F3A, F3B], axis=0)
    NI3 = np.concatenate([I3A, I3B], axis=0)
    MF = np.concatenate([_tiles(MA), _tiles(MB)], axis=0)
    NI = np.concatenate([_tiles(NA), _tiles(NB)], axis=0)
    out = dict(MF3=MF3, NI3=NI3, MF=MF, NI=NI, M0=np.stack([M0, N0]), CSF=CSF, CST=CST, CSF3=CSF3, CST3=CST3, P1=P1)
    return {k: v.astype(np.float32).astype(BF) for k, v in out.items()}

_K = _consts()

def _add(a, b):
    if a[1] == b[1]: return (a[0] + b[0], a[1])
    if a[1] > 0: return (a[0] - b[0], 1)
    return (b[0] - a[0], 1)
def _neg(a): return (a[0], -a[1])
def _sub(a, b): return _add(a, _neg(b))
def _mulc(a, c): return (a[0] * float(c * a[1]), 1)
def _val(a): return a[0] if a[1] > 0 else -a[0]
def _pos(x): return (x, 1)

C16 = [float(np.cos(2 * np.pi * k / 16)) for k in range(16)]
S16 = [float(np.sin(2 * np.pi * k / 16)) for k in range(16)]
RH = float(np.sqrt(0.5))

def _tw(re, im, k, sign):
    k = k % 16
    kk = k if sign > 0 else (16 - k) % 16
    if kk == 0: return re, im
    if kk == 4: return _neg(im), re
    if kk == 8: return _neg(re), _neg(im)
    if kk == 12: return im, _neg(re)
    if kk == 2:  return _mulc(_sub(re, im), RH), _mulc(_add(re, im), RH)
    if kk == 6:  return _mulc(_add(re, im), -RH), _mulc(_sub(re, im), RH)
    if kk == 10: return _mulc(_sub(im, re), RH), _mulc(_add(re, im), -RH)
    if kk == 14: return _mulc(_add(re, im), RH), _mulc(_sub(im, re), RH)
    c, s = C16[kk], S16[kk]
    return _sub(_mulc(re, c), _mulc(im, s)), _add(_mulc(re, s), _mulc(im, c))

def _dft4(x, sign):
    (a_r, a_i), (b_r, b_i), (c_r, c_i), (d_r, d_i) = x
    s0r, s0i = _add(a_r, c_r), _add(a_i, c_i)
    s1r, s1i = _sub(a_r, c_r), _sub(a_i, c_i)
    s2r, s2i = _add(b_r, d_r), _add(b_i, d_i)
    s3r, s3i = _sub(b_r, d_r), _sub(b_i, d_i)
    X0 = (_add(s0r, s2r), _add(s0i, s2i))
    X2 = (_sub(s0r, s2r), _sub(s0i, s2i))
    if sign < 0:
        X1 = (_add(s1r, s3i), _sub(s1i, s3r))
        X3 = (_sub(s1r, s3i), _add(s1i, s3r))
    else:
        X1 = (_sub(s1r, s3i), _add(s1i, s3r))
        X3 = (_add(s1r, s3i), _sub(s1i, s3r))
    return [X0, X1, X2, X3]

def _fft16(x, sign):
    x = [(_pos(r), _pos(i)) for r, i in x]
    inner = []
    for n1 in range(4):
        y = _dft4([x[n1 + 4 * n2] for n2 in range(4)], sign)
        inner.append([_tw(y[k2][0], y[k2][1], n1 * k2, sign) for k2 in range(4)])
    out = [None] * 16
    for k2 in range(4):
        z = _dft4([inner[n1][k2] for n1 in range(4)], sign)
        for k1 in range(4):
            out[k2 + 4 * k1] = z[k1]
    return out

def _rfft16(x):
    x = [_pos(v) for v in x]
    y0, y2, y1 = [], [], []
    for n1 in range(4):
        a, b, c, d = x[n1], x[n1 + 4], x[n1 + 8], x[n1 + 12]
        s0, s1, s2, s3 = _add(a, c), _sub(a, c), _add(b, d), _sub(b, d)
        y0.append(_add(s0, s2)); y2.append(_sub(s0, s2)); y1.append((s1, _neg(s3)))
    out = {}
    a, b, c, d = y0
    s0, s1, s2, s3 = _add(a, c), _sub(a, c), _add(b, d), _sub(b, d)
    out[0] = (_add(s0, s2), None); out[8] = (_sub(s0, s2), None); out[4] = (s1, _neg(s3))
    u0, u1, u2, u3 = y2
    p = _mulc(_sub(u1, u3), RH); qv = _mulc(_add(u1, u3), RH)
    out[2] = (_add(u0, p), _neg(_add(u2, qv)))
    out[6] = (_sub(u0, p), _sub(u2, qv))
    t = [_tw(y1[n][0], y1[n][1], n, -1) for n in range(4)]
    z = _dft4(t, -1)
    out[1] = z[0]; out[5] = z[1]
    out[7] = (z[2][0], _neg(z[2][1])); out[3] = (z[3][0], _neg(z[3][1]))
    return out

def _irfft16(B0, B8, P, Q):
    out = [None] * 16
    s, dlt = _add(B0, B8), _sub(B0, B8)
    f0 = [_add(s, P[4]), _sub(dlt, Q[4]), _sub(s, P[4]), _add(dlt, Q[4])]
    m, n = _sub(P[2], P[6]), _add(Q[2], Q[6])
    g = [_add(P[2], P[6]), _mulc(_sub(m, n), RH), _sub(Q[6], Q[2]), _mulc(_add(m, n), -RH)]
    V = [(P[1], Q[1]), (P[5], Q[5]), (P[7], _neg(Q[7])), (P[3], _neg(Q[3]))]
    U = _dft4(V, +1)
    for a in range(8):
        ur, ui = U[a % 4]
        if a == 0: h = ur
        elif a == 4: h = _neg(ui)
        else: h = _sub(_mulc(ur, C16[a]), _mulc(ui, S16[a]))
        base = _add(f0[a % 4], g[a % 4]) if a < 4 else _sub(f0[a % 4], g[a % 4])
        out[a] = _add(base, h)
        out[a + 8] = _sub(base, h)
    return out

K5 = float((np.cos(2 * np.pi / 5) - np.cos(4 * np.pi / 5)) / 2)
S51 = float(np.sin(2 * np.pi / 5))
K21 = float(np.sin(4 * np.pi / 5) / np.sin(2 * np.pi / 5))

def _gelu(h, fold=False):
    c0 = 0.7978845608028654
    u = h * (c0 + (c0 * 0.044715) * (h * h))
    if fold:
        return h * (1.0 + jnp.tanh(u))
    return (0.5 * h) * (1.0 + jnp.tanh(u))

def sched_b(n, final):
    o = [("T1", 0), ("T2d", 0), ("T2p", 0)]
    for j in range(n):
        if not final and j > 0: o += [("H1", j - 1)]
        if j + 1 < n: o += [("T1", j + 1)]
        o.append(("M1", j))
        if not final and j > 0: o += [("H2", j - 1)]
        if j + 1 < n: o += [("T2d", j + 1)]
        o.append(("M2", j))
        if j + 1 < n: o += [("T2p", j + 1)]
    if not final: o += [("H1", n - 1), ("H2", n - 1)]
    return o

def sched_e(n, final):
    o = [("T1", 0), ("T2d", 0), ("T2p", 0)]
    for j in range(n):
        if not final and j > 0: o += [("H1", j - 1)]
        o.append(("M1", j))
        if not final and j > 0: o += [("H2", j - 1)]
        if j + 1 < n: o += [("T1", j + 1)]
        o.append(("M2a", j))
        if j + 1 < n: o += [("T2d", j + 1)]
        o.append(("M2b", j))
        if j + 1 < n: o += [("T2p", j + 1)]
    if not final: o += [("H1", n - 1), ("H2", n - 1)]
    return o

def sched_g(n, final):
    o = [("T1", 0), ("T2d", 0), ("T2p", 0)]
    for j in range(n):
        if not final and j > 0: o += [("H1", j - 1)]
        o.append(("M1", j))
        if not final and j > 0: o += [("H2", j - 1)]
        o.append(("M2", j))
        if j + 1 < n: o += [("T1", j + 1), ("T2d", j + 1), ("T2p", j + 1)]
    if not final: o += [("H1", n - 1), ("H2", n - 1)]
    return o

def mk_sched(pattern):
    toks = pattern.split()
    def f(n, final):
        o = [("T1", 0), ("T2d", 0), ("T2p", 0)]
        for j in range(n):
            for t in toks:
                if t[-1] == "-":
                    if not final and j > 0: o.append((t[:-1], j - 1))
                elif t[-1] == "+":
                    if j + 1 < n: o.append((t[:-1], j + 1))
                else:
                    o.append((t, j))
        if not final: o += [("H1", n - 1), ("H2", n - 1)]
        return o
    return f

SCHEDS = dict(b=sched_b, e=sched_e, g=sched_g)

def make_kernel(chunks=(4, 4, 4, 4), sched="b", ln="two", smode="two", flags=None, split2=3, RB=16, scopes=False, m2n=False, gt=0, dt=1, start_mode=0, NXD=4, tag=False, xp=(1, 3, 4, 4, 4), splitw=True, smul=3, csplit=8, wq=(9, 9), bars=(), d3=(0, 0, 0), gfold=False, gateT=-1, gateH=-1):
    if isinstance(sched, str): sched = SCHEDS[sched] if sched in SCHEDS else mk_sched(sched)
    NCH = len(chunks)
    assert sum(chunks) == 16
    G0 = [sum(chunks[:j]) for j in range(NCH)]
    f32, bf16 = jnp.float32, jnp.bfloat16
    NT = (((1,), (1,)), ((), ()))

    def kernel(x_hbm, wr_hbm, wi_hbm, w1_hbm, b1_hbm, w2_hbm, b2_hbm,
               mf_hbm, ni_hbm, m0_hbm, csf_hbm, p1_hbm, mf3_hbm, ni3_hbm,
               o_hbm,
               xst, wr_v, wi_v, wrl_v, wil_v, w1_v, b1_v, w2_v, b2_v, mf_v, ni_v, m0_v, csf_v, p1_v, mf3_v, ni3_v,
               xs, ybuf, zsb, bbuf, wc, zbuf, abuf, xnbuf, gbuf, ost, dum, sems, osem):
        def dot(a, b):
            return jnp.dot(a, b, preferred_element_type=f32)
        def cat1(parts):
            return jnp.concatenate(parts, axis=1)
        def cat0(parts):
            return jnp.concatenate(parts, axis=0)
        u32 = jnp.uint32
        class B16:
            def __init__(self, ref): self.ref = ref
            def ld(self, lead, r0, n):
                return pltpu.bitcast(self.ref[(*lead, slice(r0 // 2, (r0 + n) // 2), slice(None))], bf16)
            def ldg(self, lead, r0, n, gate):
                v = self.ref[(*lead, slice(r0 // 2, (r0 + n) // 2), slice(None))]
                if gate is not None:
                    v = jnp.concatenate([v[0:8] | gate, v[8:]], axis=0)
                return pltpu.bitcast(v, bf16)
            def st(self, lead, r0, val):
                n = val.shape[0]
                self.ref[(*lead, slice(r0 // 2, (r0 + n) // 2), slice(None))] = pltpu.bitcast(val.astype(bf16), u32)
        W1, W2 = B16(w1_v.bitcast(u32)), B16(w2_v.bitcast(u32))
        MF_, NI_, M0_, CS_, P1_ = B16(mf_v.bitcast(u32)), B16(ni_v.bitcast(u32)), B16(m0_v.bitcast(u32)), B16(csf_v.bitcast(u32)), B16(p1_v.bitcast(u32))
        ZB, AB, XN, ZS = B16(zbuf), B16(abuf), B16(xnbuf), B16(zsb)
        MF3_, NI3_ = B16(mf3_v.bitcast(u32)), B16(ni3_v.bitcast(u32))
        si = iter(range(1000))
        def start(src, dst):
            cp = pltpu.make_async_copy(src, dst, sems.at[next(si)])
            cp.start()
            return cp
        XP0 = [sum(xp[:i]) for i in range(len(xp))]
        cps = {}
        def issue(*names):
            for nm in names:
                if nm[0] == "x":
                    i = int(nm[1:])
                    lo, hi = 8 * XP0[i], 8 * (XP0[i] + xp[i])
                    cps[nm] = start(x_hbm.at[:, lo:hi], xst.at[:, lo:hi])
                elif nm == "mf":
                    cps[nm] = ([start(mf_hbm, mf_v)] if not d3[0] else []) + ([start(mf3_hbm, mf3_v)] if d3[0] else [])
                elif nm == "mfb":
                    cps[nm] = ([start(mf_hbm, mf_v)] if (d3[0] and not d3[1]) else []) + ([start(mf3_hbm, mf3_v)] if (d3[1] and not d3[0]) else [])
                elif nm == "ni":
                    cps[nm] = [start(ni3_hbm, ni3_v)] if d3[2] else [start(ni_hbm, ni_v)]
                elif nm in ("wr", "wi"):
                    src, dst, lastv = (wr_hbm, wr_v, wrl_v) if nm == "wr" else (wi_hbm, wi_v, wil_v)
                    cps[nm] = [start(src.at[0:320, 128 * m:128 * m + 128], dst.at[m]) for m in range(16)] + [start(src.at[320:321, :], lastv)]
                elif nm in ("csf0", "csf1"):
                    hh = int(nm[-1])
                    cps[nm] = start(csf_hbm.at[8 * hh:8 * hh + 8], csf_v.at[8 * hh:8 * hh + 8])
                elif nm == "w1":
                    cps[nm] = [start(w1_hbm.at[:, 128 * p:128 * p + 128], w1_v.at[p]) for p in range(5)]
                elif nm == "w2":
                    cps[nm] = [start(w2_hbm.at[:, 128 * p:128 * p + 128], w2_v.at[p]) for p in range(5)]
                else:
                    src, dst = dict(mf=(mf_hbm, mf_v), m0=(m0_hbm, m0_v), p1=(p1_hbm, p1_v),
                                    csf=(csf_hbm, csf_v), ni=(ni_hbm, ni_v), b1=(b1_hbm, b1_v), b2=(b2_hbm, b2_v))[nm]
                    cps[nm] = start(src, dst)
        def wait(*names):
            for nm in names:
                c = cps[nm]
                for cc in (c if isinstance(c, list) else [c]):
                    cc.wait()

        lane8 = lax.broadcasted_iota(jnp.int32, (8, 128), 1)
        sF8 = jnp.where(lane8 < 64, 1.0, -1.0).astype(f32)
        lane128 = lax.broadcasted_iota(jnp.int32, (128, 128), 1)
        sF128 = jnp.where(lane128 < 64, 1.0, -1.0).astype(f32)
        def rollsg8(v):
            return pltpu.roll(v, 64, 1) * sF8

        def load_x(i):
            for gp in range(XP0[i], XP0[i] + xp[i]):
                xs[128 * gp:128 * gp + 128, :] = xst[:, 8 * gp:8 * gp + 8, :].astype(f32).reshape(128, D)

        def stats(s1, s2, eps=1e-5):
            m = jnp.sum(s1, axis=-1, keepdims=True) * (1.0 / D)
            ex2 = jnp.sum(s2, axis=-1, keepdims=True) * (1.0 / D)
            r = lax.rsqrt(jnp.maximum(ex2 - m * m, 0.0) + eps)
            return m, r

        def H1rows(r0, n, m3):
            x = xs[r0:r0 + n, :]
            x0, x1, x2, x3, x4 = [x[:, 128 * p:128 * (p + 1)] for p in range(5)]
            t1, t2, t3, t4 = x1 + x4, x2 + x3, x1 - x4, x2 - x3
            u, v = t1 + t2, t1 - t2
            z0 = x0 + u
            if ln == "one":
                m, r = stats(z0, x0 * x0 + x1 * x1 + x2 * x2 + x3 * x3 + x4 * x4)
                z0 = z0 - 5.0 * m
            else:
                m = jnp.sum(z0, axis=-1, keepdims=True) * (1.0 / D)
                xc = [xx - m for xx in (x0, x1, x2, x3, x4)]
                var = jnp.sum(xc[0] * xc[0] + xc[1] * xc[1] + xc[2] * xc[2] + xc[3] * xc[3] + xc[4] * xc[4], axis=-1, keepdims=True) * (1.0 / D)
                r = lax.rsqrt(var + 1e-5)
                z0 = z0 - 5.0 * m
            mm = x0 - 0.25 * u
            nn = K5 * v
            zs = (z0, mm + nn, t3 + K21 * t4, mm - nn, K21 * t3 - t4)
            zs = [z * r for z in zs]
            for p in range(5):
                ZB.st((p,), r0, zs[p])
            if m3:
                ZB.st((5,), r0, zs[1] - S51 * zs[2])
                ZB.st((6,), r0, zs[3] - S51 * zs[4])

        def H1(j):
            for rb in range(chunks[j] * 128 // RB):
                H1rows(G0[j] * 128 + RB * rb, RB, d3[1])

        def H2(j):
            for gp in range(G0[j], G0[j] + chunks[j]):
                H2one(gp, d3[1])

        def H2one(gp, m3):
            if True:
                r = 128 * gp
                for t in range(2):
                    if m3:
                        k1 = dot(ZB.ld((5 + t,), r, 128), MF3_.ld((3 * t,), 0, 128))
                        k2 = dot(ZB.ld((2 + 2 * t,), r, 128), MF3_.ld((3 * t + 1,), 0, 128))
                        k3 = dot(ZB.ld((1 + 2 * t,), r, 128), MF3_.ld((3 * t + 2,), 0, 128))
                        Ur, Ui = k1 - k2, (k1 - k3) * sF128
                        ins = [(Ur[8 * a:8 * a + 8], Ui[8 * a:8 * a + 8]) for a in range(16)]
                    else:
                        z = cat1([ZB.ld((1 + 2 * t,), r, 128), ZB.ld((2 + 2 * t,), r, 128)])
                        U = dot(z, cat1([MF_.ld((2 * t,), 0, 256), MF_.ld((2 * t + 1,), 0, 256)]))
                        ins = [(U[8 * a:8 * a + 8, 0:128], U[8 * a:8 * a + 8, 128:256]) for a in range(16)]
                    outs = _fft16(ins, -1)
                    for c in range(16):
                        ybuf[c, 8 * gp:8 * gp + 8, 128 * t:128 * t + 128] = _val(outs[c][0])
                        ybuf[c, 128 + 8 * gp:128 + 8 * gp + 8, 128 * t:128 * t + 128] = _val(outs[c][1])
                U = dot(ZB.ld((0,), r, 128), M0_.ld((0,), 0, 128))
                o = _rfft16([U[8 * a:8 * a + 8, :] for a in range(16)])
                def st(c, T, Tp):
                    ybuf[c, 8 * gp:8 * gp + 8, 256:384] = _val(T)
                    ybuf[c, 128 + 8 * gp:128 + 8 * gp + 8, 256:384] = _val(Tp)
                for c in (0, 8):
                    Rc = o[c][0]
                    st(c, Rc, (rollsg8(Rc[0]), Rc[1]))
                for c in range(1, 8):
                    Rc, Ic = o[c]
                    rt = (rollsg8(Rc[0]), Rc[1]); it = (rollsg8(Ic[0]), Ic[1])
                    st(c, _sub(Rc, it), _add(rt, Ic))
                    st(16 - c, _add(Rc, it), _sub(rt, Ic))

        def wprep(h):
            wv = (wr_v, wi_v)[h].bitcast(u32)
            lastv = (wrl_v, wil_v)[h]
            sub0 = lax.broadcasted_iota(jnp.int32, (8, 128), 0) == 0
            LO, HI = jnp.uint32(0xFFFF), jnp.uint32(0xFFFF0000)
            for m in range(16):
                a = {k: [] for k in range(5)}
                for ig in range(4):
                    v = [wv[m, pl.ds(r0 + 40 * ig, 8, stride=5), :] for r0 in range(5)]
                    a[1].append((v[0] >> 16) | (v[3] << 16))
                    a[4].append((v[2] & LO) | (v[4] & HI))
                    a[2].append((v[1] & LO) | (v[3] & HI))
                    a[3].append((v[1] >> 16) | (v[4] << 16))
                    a[0].append((v[0] & LO) | (v[2] & HI))
                r320 = pltpu.bitcast(jnp.broadcast_to(lastv[:, 128 * m:128 * m + 128].astype(f32), (8, 128)), u32) >> 16
                a[0][0] = jnp.where(sub0, (a[0][0] & HI) | r320, a[0][0])
                T = pltpu.bitcast(cat0(a[1] + a[4] + a[2] + a[3] + a[0] + a[0]), bf16)
                O = lax.dot_general(P1_.ld((), 0, 128), T, NT, preferred_element_type=f32)
                for c in range(16):
                    wc[c, 128 * h + 8 * m:128 * h + 8 * m + 8, :] = O[8 * c:8 * c + 8, :]

        def mix(c, Xr, Xi):
            Wr, Wi = wc[c, 0:128, :], wc[c, 128:256, :]
            return Xr * Wr - Xi * Wi, Xr * Wi + Xi * Wr
        def sfwd(c):
            if smul == 3:
                Yr, Yi = ybuf[c, 0:128, :], ybuf[c, 128:256, :]
                k1 = dot(CS_.ld((c,), 0, 128), (Yr + Yi).astype(bf16))
                k2 = dot(CS_.ld((c,), 128, 128), Yi.astype(bf16))
                k3 = dot(CS_.ld((c,), 256, 128), Yr[:, 0:256].astype(bf16))
                Xr = k1 - k2
                Xi = cat1([k1[:, 0:256] - k3, pltpu.roll(Xr[:, 256:384], 64, 1) * sF128])
                Zr, Zi = mix(c, Xr, Xi)
                return cat0([Zr + Zi, Zi, Zr]).astype(bf16)
            L = csf_v[c]
            Yr = ybuf[c, 0:128, :].astype(bf16)
            Yi = ybuf[c, 128:256, :].astype(bf16)
            P = dot(L, Yr[:, 0:256])
            Q = dot(L, Yi[:, 0:256])
            X0 = dot(L[0:128], Yr[:, 256:384]) + dot(L[128:256], Yi[:, 256:384])
            Xr = cat1([P[0:128] + Q[128:256], X0])
            Xi = cat1([Q[0:128] - P[128:256], pltpu.roll(X0, 64, 1) * sF128])
            Zr, Zi = mix(c, Xr, Xi)
            return cat0([Zr, Zi]).astype(bf16)
        def sinv(c, Z):
            if smul == 3:
                TN = (((0,), (0,)), ((), ()))
                k1 = lax.dot_general(CS_.ld((c,), 0, 128), Z[0:128], TN, preferred_element_type=f32)
                k2 = lax.dot_general(CS_.ld((c,), 256, 128), Z[128:256], TN, preferred_element_type=f32)
                k3 = lax.dot_general(CS_.ld((c,), 128, 128), Z[256:384, 0:256], TN, preferred_element_type=f32)
                bbuf[c, 0:128, :] = k1 - k2
                bbuf[c, 128:256, 0:256] = k1[:, 0:256] - k3
                return
            L = cst_v[c]
            P = dot(L, Z[0:128, 0:256])
            Q = dot(L, Z[128:256, 0:256])
            bbuf[c, 0:128, 0:256] = P[0:128] - Q[128:256]
            bbuf[c, 128:256, 0:256] = Q[0:128] + P[128:256]
            bbuf[c, 0:128, 256:384] = dot(L[0:128], Z[0:128, 256:384]) - dot(L[128:256], Z[128:256, 256:384])
        TN = (((0,), (0,)), ((), ()))
        def dotT(a, b):
            return lax.dot_general(a, b, TN, preferred_element_type=f32)
        def sinv3(c):
            k1 = dotT(CS_.ld((c,), 0, 128), cat1([ZS.ld((c, t), 0, 128) for t in range(3)]))
            k2 = dotT(CS_.ld((c,), 256, 128), cat1([ZS.ld((c, t), 128, 128) for t in range(3)]))
            k3 = dotT(CS_.ld((c,), 128, 128), cat1([ZS.ld((c, t), 256, 128) for t in range(2)]))
            bbuf[c, 0:128, :] = k1 - k2
            bbuf[c, 128:256, 0:256] = k1[:, 0:256] - k3
        def sphase(first):
            if smode == "two":
                if first:
                    wait('csf')
                    issue(*post.get('csf', ()))
                for c in range(16):
                    Z = sfwd(c)
                    for t in range(3):
                        if smul == 3 and t == 2:
                            ZS.st((c, t), 0, Z[0:256, 128 * t:128 * t + 128])
                        else:
                            ZS.st((c, t), 0, Z[:, 128 * t:128 * t + 128])
                pass
                for c in range(16):
                    if smul == 3:
                        sinv3(c)
                    else:
                        sinv(c, cat1([zsb[c, t] for t in range(3)]))
            else:
                if first:
                    wait('csf0')
                    issue(*post.get('csf', ()))
                Z = sfwd(0)
                for c in range(15):
                    if first and c == csplit - 1:
                        wait('csf1')
                        issue(*post.get('csf1', ()))
                    Zn = sfwd(c + 1)
                    sinv(c, Z)
                    Z = Zn
                sinv(15, Z)

        def T1(j):
            for gp in range(G0[j], G0[j] + chunks[j]):
                for t in range(2):
                    ins = [(bbuf[c, 8 * gp:8 * gp + 8, 128 * t:128 * (t + 1)],
                            bbuf[c, 128 + 8 * gp:128 + 8 * gp + 8, 128 * t:128 * (t + 1)]) for c in range(16)]
                    outs = _fft16(ins, +1)
                    if d3[2]:
                        for a in range(0, 16, 2):
                            r = 128 * gp + 8 * a
                            ar = cat0([_val(outs[a][0]), _val(outs[a + 1][0])])
                            ai = cat0([_val(outs[a][1]) * sF8, _val(outs[a + 1][1]) * sF8])
                            AB.st((2 * t,), r, ar); AB.st((2 * t + 1,), r, ai); AB.st((5 + t,), r, ar + ai)
                    else:
                      for h in range(2):
                        for a in range(0, 16, 2):
                            r = 128 * gp + 8 * a
                            AB.st((2 * t + h,), r, cat0([_val(outs[a][h]), _val(outs[a + 1][h])]))
                Bv = [_pos(bbuf[c, 8 * gp:8 * gp + 8, 256:384]) for c in range(16)]
                P = {c: _add(Bv[c], Bv[16 - c]) for c in range(1, 8)}
                Q = {c: _pos(rollsg8(_val(_sub(Bv[c], Bv[16 - c])))) for c in range(1, 8)}
                outs = _irfft16(Bv[0], Bv[8], P, Q)
                for a in range(0, 16, 2):
                    r = 128 * gp + 8 * a
                    AB.st((4,), r, cat0([_val(outs[a]), _val(outs[a + 1])]))

        vals = {}
        def T2d(j):
            res = []
            gate = vals.pop(("gate", j - 1), None)
            for gp in range(G0[j], G0[j] + chunks[j]):
                r0 = 128 * gp
                if d3[2]:
                    TT = []
                    for t in range(2):
                        k1 = dot(AB.ldg((5 + t,), r0, 128, gate), NI3_.ld((3 * t,), 0, 128))
                        k2 = dot(AB.ldg((2 * t + 1,), r0, 128, gate), NI3_.ld((3 * t + 1,), 0, 128))
                        k3 = dot(AB.ldg((2 * t,), r0, 128, gate), NI3_.ld((3 * t + 2,), 0, 128))
                        TT.append(cat1([k1 - k2, k1 + k3]))
                    TA, TB = TT
                else:
                    TA = dot(cat1([AB.ld((0,), r0, 128), AB.ld((1,), r0, 128)]), cat1([NI_.ld((0,), 0, 256), NI_.ld((1,), 0, 256)]))
                    TB = dot(cat1([AB.ld((2,), r0, 128), AB.ld((3,), r0, 128)]), cat1([NI_.ld((2,), 0, 256), NI_.ld((3,), 0, 256)]))
                T0 = dot(AB.ldg((4,), r0, 128, gate), M0_.ld((1,), 0, 128))
                res.append((TA, TB, T0))
            vals["T", j] = res

        def T2p(j):
            for gi, (TA, TB, T0) in enumerate(vals.pop(("T", j))):
                r0 = 128 * (G0[j] + gi)
                for rb in range(128 // RB):
                    lo, hi = RB * rb, RB * rb + RB
                    t0, t1r, t1i, t2r, t2i = T0[lo:hi], TA[lo:hi, 0:128], TA[lo:hi, 128:256], TB[lo:hi, 0:128], TB[lo:hi, 128:256]
                    u, v = t1r + t2r, t1r - t2r
                    mm, nn = t0 - 0.25 * u, K5 * v
                    E1, E2 = mm + nn, mm - nn
                    if d3[2]:
                        O1 = S51 * t1i + (S51 * K21) * t2i
                        O2 = (S51 * K21) * t1i - S51 * t2i
                    else:
                        O1 = t1i + K21 * t2i
                        O2 = K21 * t1i - t2i
                    x = xs[r0 + lo:r0 + hi, :]
                    x1 = [x[:, 0:128] + (t0 + u), x[:, 128:256] + (E1 - O1), x[:, 256:384] + (E2 - O2),
                          x[:, 384:512] + (E2 + O2), x[:, 512:640] + (E1 + O1)]
                    xs[r0 + lo:r0 + hi, :] = cat1(x1)
                    if ln == "one":
                        m, r = stats(x1[0] + x1[1] + x1[2] + x1[3] + x1[4],
                                     x1[0] * x1[0] + x1[1] * x1[1] + x1[2] * x1[2] + x1[3] * x1[3] + x1[4] * x1[4], 1e-5 * (1.0001 if tag else 1.0))
                        xc = [xx - m for xx in x1]
                    else:
                        m = jnp.sum(x1[0] + x1[1] + x1[2] + x1[3] + x1[4], axis=-1, keepdims=True) * (1.0 / D)
                        xc = [xx - m for xx in x1]
                        var = jnp.sum(xc[0] * xc[0] + xc[1] * xc[1] + xc[2] * xc[2] + xc[3] * xc[3] + xc[4] * xc[4], axis=-1, keepdims=True) * (1.0 / D)
                        r = lax.rsqrt(var + 1e-5)
                    for p in range(5):
                        XN.st((p,), r0 + lo, xc[p] * r)

        NTL = (F + 127) // 128
        def M1(j):
            r, M = G0[j] * 128, chunks[j] * 128
            if gt == 0:
                xn = cat1([XN.ld((p,), r, M) for p in range(5)])
                h = lax.dot_general(xn, cat1([W1.ld((p,), 0, F) for p in range(5)]), NT, preferred_element_type=f32)
                h = h + b1_v[...].astype(f32).reshape(1, F)
                vals["G", j] = _gelu(h, gfold).astype(bf16)
            else:
                for n0 in range(0, NTL, gt):
                    c0, c1 = 128 * n0, min(F, 128 * (n0 + gt))
                    xn = cat1([xnbuf[p, r:r + M, :] for p in range(5)])
                    h = lax.dot_general(xn, cat1([w1_v[p, c0:c1, :] for p in range(5)]), NT, preferred_element_type=f32)
                    h = h + b1_v[c0:c1].astype(f32).reshape(1, c1 - c0)
                    g = _gelu(h).astype(bf16)
                    for n in range(n0, min(NTL, n0 + gt)):
                        lo, hi = 128 * (n - n0), min(128 * (n - n0 + 1), c1 - c0)
                        gbuf[n, r:r + M, 0:hi - lo] = g[:, lo:hi]

        def M1part(j, n0, n1):
            r, M = G0[j] * 128, chunks[j] * 128
            c0, c1 = 128 * n0, min(F, 128 * n1)
            xn = cat1([XN.ld((p,), r, M) for p in range(5)])
            h = lax.dot_general(xn, cat1([W1.ld((p,), c0, c1 - c0) for p in range(5)]), NT, preferred_element_type=f32)
            h = h + b1_v[c0:c1].astype(f32).reshape(1, c1 - c0)
            vals.setdefault(("Gp", j), []).append(_gelu(h, gfold).astype(bf16))
            if n1 >= NTL:
                vals["G", j] = cat1(vals.pop(("Gp", j)))

        b2f = lambda p0, p1: b2_v[...].astype(f32).reshape(1, D)[:, 128 * p0:128 * p1]
        def loadG(r, M):
            return cat1([gbuf[n, r:r + M, :] for n in range(NTL - 1)] + [gbuf[NTL - 1, r:r + M, 0:F - 128 * (NTL - 1)]])
        def M2part(j, final, p0, p1, last):
            r, M = G0[j] * 128, chunks[j] * 128
            g = vals["G", j] if gt == 0 else loadG(r, M)
            dd = dot(g, cat1([W2.ld((p,), 0, F) for p in range(p0, p1)]))
            x2 = xs[r:r + M, 128 * p0:128 * p1] + (0.5 * dd if gfold else dd) + b2f(p0, p1)
            if p0 == gateT:
                vals["gate", j] = pltpu.bitcast(jnp.minimum(jnp.abs(x2[0:8, 0:128]), 0.0), u32)
            if not final:
                xs[r:r + M, 128 * p0:128 * p1] = x2
            else:
                for a in range(16):
                    v = cat0([x2[128 * gg + 8 * a:128 * gg + 8 * a + 8, :] for gg in range(chunks[j])])
                    ost[a, 8 * G0[j]:8 * (G0[j] + chunks[j]), 128 * p0:128 * p1] = v.astype(bf16)
                if last:
                    lo, hi = 8 * G0[j], 8 * (G0[j] + chunks[j])
                    pltpu.make_async_copy(ost.at[:, lo:hi], o_hbm.at[:, lo:hi], osem.at[j]).start()
            if last and gt == 0: vals.pop(("G", j))

        def M2parts(j, final, p0, p1, last):
            if m2n:
                for p in range(p0, p1, dt):
                    M2part(j, final, p, min(p1, p + dt), last and p + dt >= p1)
            else:
                M2part(j, final, p0, p1, last)

        import contextlib
        sc = (lambda n: jax.named_scope(n)) if scopes else (lambda n: contextlib.nullcontext())
        def piece(i):
            load_x(i)
            for gp in range(XP0[i], XP0[i] + xp[i]):
                for rb in range(128 // RB):
                    H1rows(128 * gp + RB * rb, RB, d3[0])
            for gp in range(XP0[i], XP0[i] + xp[i]):
                H2one(gp, d3[0])
        NP = len(xp)
        barcp = {}
        def bar_issue():
            for i, nm in enumerate(bars):
                barcp[nm] = start(p1_hbm, dum.at[i])
        def bar(nm):
            if nm in barcp: barcp.pop(nm).wait()
        if start_mode == 0:
            issue("x0", "mf", "m0", *["x%d" % i for i in range(1, NP)], "p1", "wr", "wi", "csf0", "csf1", "ni", "mfb", "w1", "b1", "w2", "b2")
            plan = {}; post = {}
            bar_issue()
        elif start_mode == 1:
            issue("x0", "mf", "m0", *["x%d" % i for i in range(1, NP - 1)], "p1", "wr", "x%d" % (NP - 1), "wi", "csf0", "csf1", "ni", "mfb", "w1", "b1", "w2", "b2")
            plan = {}; post = {}
        elif start_mode == 4:
            issue("x0", "mf", "m0", "x1")
            plan = {0: ("x2", "x3"), 1: ("x4", "p1", "wr"), 2: ("wi",), 3: ("csf0",), 4: ("csf1", "ni")}
            post = {"wi": ("w1", "b1"), "csf": ("w2", "b2")}
        elif start_mode == 5:
            issue("x0", "mf", "m0", "x1")
            plan = {0: ("x2", "x3"), 1: ("x4", "p1"), 2: ("wr",), 3: ("wi",), 4: ("csf0",)}
            post = {"wr": ("csf1", "ni"), "wi": ("w1", "b1"), "csf": ("w2", "b2")}
        elif start_mode == 7:
            issue("x0", "mf", "m0", "x1")
            plan = {0: ("x2", "p1", "wr"), 1: ("x3",), 2: ("x4", "wi"), 3: ("csf0",), 4: ("csf1", "ni")}
            post = {"wi": ("w1", "b1"), "csf": ("w2", "b2")}
        elif start_mode == 8:
            issue("x0", "mf", "m0", "x1", "x2")
            plan = {0: ("p1", "wr"), 1: ("x3", "x4"), 2: ("wi",), 3: ("csf0",), 4: ("csf1", "ni")}
            post = {"wi": ("w1", "b1"), "csf": ("w2", "b2")}
        elif start_mode == 6:
            issue("x0", "mf", "m0", "x1")
            plan = {0: ("x2", "x3"), 1: ("x4", "p1", "wr"), 2: ("wi",), 3: ("csf0",), 4: ("csf1",)}
            post = {"wr": ("ni", "w1", "b1"), "wi": ("w2", "b2")}
        with sc("head0"):
            for i in range(NP):
                with sc("wx%d" % i):
                    wait("x%d" % i)
                    if i == 0: wait("mf", "m0")
                    if i == wq[0]: wait("p1", "wr")
                    if i == wq[1]: wait("wi")
                issue(*plan.get(i, ()))
                if i == wq[0]: issue(*post.get("wr", ()))
                if i == wq[1]: issue(*post.get("wi", ()))
                with sc("p%d" % i):
                    piece(i)
                    if i == wq[0]: wprep(0)
                    if i == wq[1]: wprep(1)
        with sc("wprep"):
            if wq[0] >= NP:
                with sc("w_wr"):
                    wait("p1", "wr")
                issue(*post.get("wr", ()))
                wprep(0)
            if wq[1] >= NP:
                with sc("w_wi"):
                    wait("wi")
                issue(*post.get("wi", ()))
                wprep(1)
        with sc("s1"):
            sphase(True)
        if splitw:
            with sc("w_ni"):
                wait("ni", "mfb")
        else:
            with sc("w_w12"):
                wait("ni", "w1", "b1", "w2", "b2")
        waited = set()
        def need(*names):
            if not splitw: return
            nn = [n for n in names if n not in waited]
            if nn:
                with sc("w_" + nn[0]):
                    wait(*nn)
                waited.update(nn)
        for layer in range(2):
            final = layer == 1
            with sc("mlp%d" % layer):
              for name, j in sched(NCH, final):
                if name == "M1":
                    need("w1", "b1"); M1(j)
                elif name == "M2":
                    need("w2", "b2"); M2parts(j, final, 0, 5, True)
                elif name.startswith("M1:"):
                    need("w1", "b1"); _, a, b = name.split(":"); M1part(j, int(a), int(b))
                elif name.startswith("M2:"):
                    need("w2", "b2"); _, a, b = name.split(":"); M2parts(j, final, int(a), int(b), int(b) == 5)
                elif name == "M2a": M2parts(j, final, 0, split2, False)
                elif name == "M2b": M2parts(j, final, split2, 5, True)
                elif name == "T1": T1(j)
                elif name == "T2d": T2d(j)
                elif name == "T2p": T2p(j)
                elif name == "H1": H1(j)
                elif name == "H2": H2(j)
                else: raise ValueError(name)
            if not final:
                bar("pre_s2")
                with sc("s2"):
                    sphase(False)
                bar("post_s2")
        with sc("outwait"):
          for j in range(NCH):
            lo, hi = 8 * G0[j], 8 * (G0[j] + chunks[j])
            pltpu.make_async_copy(ost.at[:, lo:hi], o_hbm.at[:, lo:hi], osem.at[j]).wait()

    def fn(A_x, A_w_r, A_w_i, B_x, B_w1, B_b1, B_w2, B_b2):
        x3 = A_x.reshape(16, 128, D)
        hbm = pl.BlockSpec(memory_space=pltpu.HBM)
        V = pltpu.VMEM
        scratch = [
            V((16, 128, D), bf16), V((16, 320, 128), bf16), V((16, 320, 128), bf16), V((1, S), bf16), V((1, S), bf16),
            V((5, F, 128), bf16), V((F,), bf16), V((5, F, 128), bf16), V((D,), bf16),
            V((4, 256, 128), bf16), V((4, 256, 128), bf16), V((2, 128, 128), bf16),
            V((16, 384, 128), bf16), V((128, 128), bf16), V((6, 128, 128), bf16), V((6, 128, 128), bf16),
            V((S, D), f32), V((16, 256, 384), f32), V((16, 3, 64 * (6 - smul), 128), jnp.uint32), V((16, 256, 384), f32),
            V((16, 256, 384), f32),
            V((7, S // 2, 128), jnp.uint32), V((7, S // 2, 128), jnp.uint32), V((5, S // 2, 128), jnp.uint32),
            V((14, S, 128), bf16),
            V((16, 128, D), bf16), V((8, 128, 128), bf16),
            pltpu.SemaphoreType.DMA((80,)), pltpu.SemaphoreType.DMA((NCH,)),
        ]
        K = _K
        out = pl.pallas_call(
            kernel,
            out_shape=jax.ShapeDtypeStruct((16, 128, D), bf16),
            in_specs=[hbm] * 14,
            out_specs=hbm,
            scratch_shapes=scratch,
            compiler_params=pltpu.CompilerParams(vmem_limit_bytes=110 * 1024 * 1024, flags=flags),
        )(x3, A_w_r.T, A_w_i.T, B_w1.T, B_b1, B_w2, B_b2,
          K["MF"], K["NI"], K["M0"], K["CSF3"], K["P1"], K["MF3"], K["NI3"])
        return out.reshape(1, S, D)
    return fn


_FN = make_kernel(**dict(ln='one',chunks=(1,)*16,m2n=True,smode='skew',start_mode=0,bars=('post_s2',),d3=(1,1,1),gfold=True,sched='H1- T1+ M1 H2- M2:0:2 T2d+ M2:2:5 T2p+'))


@jax.jit
def pallas_interleave_layers__spectral_gfnet__dense_activation_gelu__prompt_kernel(
    A_x: jax.Array,
    A_w_r: jax.Array,
    A_w_i: jax.Array,
    B_x: jax.Array,
    B_w1: jax.Array,
    B_b1: jax.Array,
    B_w2: jax.Array,
    B_b2: jax.Array,
):
    return _FN(A_x, A_w_r, A_w_i, B_x, B_w1, B_b1, B_w2, B_b2)
```

```python
import numpy as np
import jax
import jax.numpy as jnp
from jax import lax
from jax.experimental import pallas as pl
from jax.experimental.pallas import tpu as pltpu
import ml_dtypes

S, D, F = 2048, 640, 1728
NMINI = 16
XPIECES = (1, 3, 4, 4, 4)
S51 = float(np.sin(2 * np.pi / 5))
K5 = float((np.cos(2 * np.pi / 5) - np.cos(4 * np.pi / 5)) / 2)
K21 = float(np.sin(4 * np.pi / 5) / np.sin(2 * np.pi / 5))


def _consts():
    e = np.arange(128)
    q = np.arange(128)
    sgn = np.where(e < 64, 1.0, -1.0)
    lA = np.where(e < 64, 1 + 5 * e, 4 + 5 * (e - 64))
    lB = np.where(e < 64, 2 + 5 * e, 3 + 5 * (e - 64))

    def three_mult(l):
        ph = 2 * np.pi * ((q[:, None] * l[None, :]) % D) / D
        c, s = np.cos(ph), sgn[None, :] * np.sin(ph)
        fwd = np.stack([c, -S51 * (c - s), c + s])
        inv = 2.0 / (S * D) * np.stack([c.T, (c + s).T, (s - c).T])
        return fwd, inv

    fA, iA = three_mult(lA)
    fB, iB = three_mult(lB)
    e0 = np.arange(64)
    l0 = np.where(e0 == 0, D // 2, 5 * e0)
    ph = 2 * np.pi * ((q[:, None] * l0[None, :]) % D) / D
    c, s = np.cos(ph), np.sin(ph)
    s = np.where(np.abs(s) < 1e-9, 0.0, s)
    cl = np.where(e0 == 0, 1.0, 2.0) / (S * D)
    M0 = np.concatenate([c, -s], axis=1)
    N0 = np.concatenate([c.T * cl[:, None], -s.T * cl[:, None]], axis=0)
    d = np.arange(128)
    CSF = np.zeros((16, 384, 128))
    CST = np.zeros((16, 384, 128))
    for cc in range(16):
        ph = 2 * np.pi * ((d[None, :] * (cc + 16 * d[:, None])) % S) / S
        C, Sn = np.cos(ph), np.sin(ph)
        CSF[cc] = np.concatenate([C, C - Sn, C + Sn], axis=0)
        CST[cc] = np.concatenate([C.T, C.T + Sn.T, C.T - Sn.T], axis=0)
    P1 = np.zeros((128, 128))
    for cc in range(16):
        for j in range(8):
            P1[8 * cc + j, 16 * j + cc] = 1.0
    out = dict(MF=np.concatenate([fA, fB]), NI=np.concatenate([iA, iB]), M0=np.stack([M0, N0]),
               CSF=CSF, CST=CST, P1=P1)
    return {k: v.astype(np.float32).astype(ml_dtypes.bfloat16) for k, v in out.items()}


_K = _consts()


def _add(a, b):
    if a[1] == b[1]:
        return (a[0] + b[0], a[1])
    if a[1] > 0:
        return (a[0] - b[0], 1)
    return (b[0] - a[0], 1)


def _neg(a):
    return (a[0], -a[1])


def _sub(a, b):
    return _add(a, _neg(b))


def _mulc(a, c):
    return (a[0] * float(c * a[1]), 1)


def _val(a):
    return a[0] if a[1] > 0 else -a[0]


def _pos(x):
    return (x, 1)


C16 = [float(np.cos(2 * np.pi * k / 16)) for k in range(16)]
S16 = [float(np.sin(2 * np.pi * k / 16)) for k in range(16)]
RH = float(np.sqrt(0.5))


def _tw(re, im, k, sign):
    k = k % 16
    kk = k if sign > 0 else (16 - k) % 16
    if kk == 0:
        return re, im
    if kk == 4:
        return _neg(im), re
    if kk == 8:
        return _neg(re), _neg(im)
    if kk == 12:
        return im, _neg(re)
    if kk == 2:
        return _mulc(_sub(re, im), RH), _mulc(_add(re, im), RH)
    if kk == 6:
        return _mulc(_add(re, im), -RH), _mulc(_sub(re, im), RH)
    if kk == 10:
        return _mulc(_sub(im, re), RH), _mulc(_add(re, im), -RH)
    if kk == 14:
        return _mulc(_add(re, im), RH), _mulc(_sub(im, re), RH)
    c, s = C16[kk], S16[kk]
    return _sub(_mulc(re, c), _mulc(im, s)), _add(_mulc(re, s), _mulc(im, c))


def _dft4(x, sign):
    (a_r, a_i), (b_r, b_i), (c_r, c_i), (d_r, d_i) = x
    s0r, s0i = _add(a_r, c_r), _add(a_i, c_i)
    s1r, s1i = _sub(a_r, c_r), _sub(a_i, c_i)
    s2r, s2i = _add(b_r, d_r), _add(b_i, d_i)
    s3r, s3i = _sub(b_r, d_r), _sub(b_i, d_i)
    X0 = (_add(s0r, s2r), _add(s0i, s2i))
    X2 = (_sub(s0r, s2r), _sub(s0i, s2i))
    if sign < 0:
        X1 = (_add(s1r, s3i), _sub(s1i, s3r))
        X3 = (_sub(s1r, s3i), _add(s1i, s3r))
    else:
        X1 = (_sub(s1r, s3i), _add(s1i, s3r))
        X3 = (_add(s1r, s3i), _sub(s1i, s3r))
    return [X0, X1, X2, X3]


def _fft16(x, sign):
    x = [(_pos(r), _pos(i)) for r, i in x]
    inner = []
    for n1 in range(4):
        y = _dft4([x[n1 + 4 * n2] for n2 in range(4)], sign)
        inner.append([_tw(y[k2][0], y[k2][1], n1 * k2, sign) for k2 in range(4)])
    out = [None] * 16
    for k2 in range(4):
        z = _dft4([inner[n1][k2] for n1 in range(4)], sign)
        for k1 in range(4):
            out[k2 + 4 * k1] = z[k1]
    return out


def _rfft16(x):
    x = [_pos(v) for v in x]
    y0, y2, y1 = [], [], []
    for n1 in range(4):
        a, b, c, d = x[n1], x[n1 + 4], x[n1 + 8], x[n1 + 12]
        s0, s1, s2, s3 = _add(a, c), _sub(a, c), _add(b, d), _sub(b, d)
        y0.append(_add(s0, s2))
        y2.append(_sub(s0, s2))
        y1.append((s1, _neg(s3)))
    out = {}
    a, b, c, d = y0
    s0, s1, s2, s3 = _add(a, c), _sub(a, c), _add(b, d), _sub(b, d)
    out[0] = (_add(s0, s2), None)
    out[8] = (_sub(s0, s2), None)
    out[4] = (s1, _neg(s3))
    u0, u1, u2, u3 = y2
    p = _mulc(_sub(u1, u3), RH)
    qv = _mulc(_add(u1, u3), RH)
    out[2] = (_add(u0, p), _neg(_add(u2, qv)))
    out[6] = (_sub(u0, p), _sub(u2, qv))
    t = [_tw(y1[n][0], y1[n][1], n, -1) for n in range(4)]
    z = _dft4(t, -1)
    out[1] = z[0]
    out[5] = z[1]
    out[7] = (z[2][0], _neg(z[2][1]))
    out[3] = (z[3][0], _neg(z[3][1]))
    return out


def _irfft16(B0, B8, P, Q):
    out = [None] * 16
    s, dlt = _add(B0, B8), _sub(B0, B8)
    f0 = [_add(s, P[4]), _sub(dlt, Q[4]), _sub(s, P[4]), _add(dlt, Q[4])]
    m, n = _sub(P[2], P[6]), _add(Q[2], Q[6])
    g = [_add(P[2], P[6]), _mulc(_sub(m, n), RH), _sub(Q[6], Q[2]), _mulc(_add(m, n), -RH)]
    V = [(P[1], Q[1]), (P[5], Q[5]), (P[7], _neg(Q[7])), (P[3], _neg(Q[3]))]
    U = _dft4(V, +1)
    for a in range(8):
        ur, ui = U[a % 4]
        if a == 0:
            h = ur
        elif a == 4:
            h = _neg(ui)
        else:
            h = _sub(_mulc(ur, C16[a]), _mulc(ui, S16[a]))
        base = _add(f0[a % 4], g[a % 4]) if a < 4 else _sub(f0[a % 4], g[a % 4])
        out[a] = _add(base, h)
        out[a + 8] = _sub(base, h)
    return out


def _gelu2(h):
    c0 = 0.7978845608028654
    u = h * (c0 + (c0 * 0.044715) * (h * h))
    return h * (1.0 + jnp.tanh(u))


f32, bf16, u32 = jnp.float32, jnp.bfloat16, jnp.uint32
NT = (((1,), (1,)), ((), ()))
TN = (((0,), (0,)), ((), ()))
FM = 128 * (F // 128)
FP = FM + 128


def _dot(a, b):
    return jnp.dot(a, b, preferred_element_type=f32)


def _cat1(parts):
    return jnp.concatenate(parts, axis=1)


def _cat0(parts):
    return jnp.concatenate(parts, axis=0)


class _B16:
    def __init__(self, raw):
        self.raw = raw
        self.words = raw.bitcast(u32)

    def ld(self, lead, r0, n):
        return pltpu.bitcast(self.words[(*lead, slice(r0 // 2, (r0 + n) // 2), slice(None))], bf16)

    def st(self, lead, r0, val):
        self.raw[(*lead, slice(r0, r0 + val.shape[0]), slice(None))] = val.astype(bf16)


def _kernel(x_hbm, wr_hbm, wi_hbm, w1_hbm, b1_hbm, w2_hbm, b2_hbm,
            mf_hbm, ni_hbm, m0_hbm, csf_hbm, cst_hbm, p1_hbm,
            o_hbm,
            xst, wr_v, wi_v, wrl_v, wil_v, w1_v, b1_v, w2_v, b2_v,
            mf_v, ni_v, m0_v, csf_v, cst_v, p1_v,
            xs, ybuf, bbuf, wc, zbuf, abuf, xnbuf, ost, sync_v, b1col, sems, osem):
    W1, W2 = _B16(w1_v), _B16(w2_v)
    MF, NI, M0, CS, CT, P1 = _B16(mf_v), _B16(ni_v), _B16(m0_v), _B16(csf_v), _B16(cst_v), _B16(p1_v)
    ZB, AB, XN = _B16(zbuf), _B16(abuf), _B16(xnbuf)

    nsem = [0]

    def start(src, dst):
        cp = pltpu.make_async_copy(src, dst, sems.at[nsem[0]])
        nsem[0] += 1
        cp.start()
        return [cp]

    def wait(*groups):
        for grp in groups:
            for cp in grp:
                cp.wait()

    xp0 = [sum(XPIECES[:i]) for i in range(len(XPIECES))]

    def x_copy(i):
        lo, hi = 8 * xp0[i], 8 * (xp0[i] + XPIECES[i])
        return start(x_hbm.at[:, lo:hi], xst.at[:, lo:hi])

    def w_copy(src, dst, last, ms):
        cps = sum([start(src.at[0:320, 128 * m:128 * m + 128], dst.at[m]) for m in ms], [])
        return cps + (start(src.at[320:321, :], last) if ms[0] == 0 else [])

    cp_x = [x_copy(0)]
    cp_mf = start(mf_hbm, mf_v)
    cp_m0 = start(m0_hbm, m0_v)
    cp_x += [x_copy(i) for i in range(1, len(XPIECES))]
    cp_p1 = start(p1_hbm, p1_v)
    lo_m, hi_m = list(range(0, 8)), list(range(8, 16))
    cp_wra = w_copy(wr_hbm, wr_v, wrl_v, lo_m)
    cp_wia = w_copy(wi_hbm, wi_v, wil_v, lo_m)
    cp_wrb = w_copy(wr_hbm, wr_v, wrl_v, hi_m)
    cp_wib = w_copy(wi_hbm, wi_v, wil_v, hi_m)
    cp_cs0 = start(csf_hbm.at[0:8], csf_v.at[0:8])
    cp_cs1 = start(csf_hbm.at[8:16], csf_v.at[8:16])
    cp_ni = start(ni_hbm, ni_v)
    cp_w1 = sum([start(w1_hbm.at[:, 128 * p:128 * p + 128], w1_v.at[p]) for p in range(5)], []) + start(b1_hbm, b1_v)
    cp_w2 = sum([start(w2_hbm.at[:, 128 * p:128 * p + 128], w2_v.at[p, 0:F]) for p in range(5)], []) + start(b2_hbm, b2_v)
    cp_cst = start(cst_hbm, cst_v)
    cp_sync = start(p1_hbm, sync_v)

    lane8 = lax.broadcasted_iota(jnp.int32, (8, 128), 1)
    sF8 = jnp.where(lane8 < 64, 1.0, -1.0).astype(f32)
    lane128 = lax.broadcasted_iota(jnp.int32, (128, 128), 1)
    sF128 = jnp.where(lane128 < 64, 1.0, -1.0).astype(f32)

    def rollsg8(v):
        return pltpu.roll(v, 64, 1) * sF8

    def stats(s1, s2):
        m = jnp.sum(s1, axis=-1, keepdims=True) * (1.0 / D)
        ex2 = jnp.sum(s2, axis=-1, keepdims=True) * (1.0 / D)
        return m, lax.rsqrt(jnp.maximum(ex2 - m * m, 0.0) + 1e-5)

    def H1(g):
        for r0 in range(128 * g, 128 * g + 128, 16):
            x = xs[r0:r0 + 16, :]
            x0, x1, x2, x3, x4 = [x[:, 128 * p:128 * (p + 1)] for p in range(5)]
            t1, t2, t3, t4 = x1 + x4, x2 + x3, x1 - x4, x2 - x3
            u, v = t1 + t2, t1 - t2
            z0 = x0 + u
            m, r = stats(z0, x0 * x0 + x1 * x1 + x2 * x2 + x3 * x3 + x4 * x4)
            z0 = z0 - 5.0 * m
            mm = x0 - 0.25 * u
            nn = K5 * v
            zs = [z * r for z in (z0, mm + nn, t3 + K21 * t4, mm - nn, K21 * t3 - t4)]
            for p in range(5):
                ZB.st((p,), r0, zs[p])
            ZB.st((5,), r0, zs[1] - S51 * zs[2])
            ZB.st((6,), r0, zs[3] - S51 * zs[4])

    def H2(g):
        r = 128 * g
        for t in range(2):
            k1 = _dot(ZB.ld((5 + t,), r, 128), MF.ld((3 * t,), 0, 128))
            k2 = _dot(ZB.ld((2 + 2 * t,), r, 128), MF.ld((3 * t + 1,), 0, 128))
            k3 = _dot(ZB.ld((1 + 2 * t,), r, 128), MF.ld((3 * t + 2,), 0, 128))
            Ur, Ui = k1 - k2, (k1 - k3) * sF128
            outs = _fft16([(Ur[8 * a:8 * a + 8], Ui[8 * a:8 * a + 8]) for a in range(16)], -1)
            for c in range(16):
                ybuf[c, 8 * g:8 * g + 8, 128 * t:128 * t + 128] = _val(outs[c][0])
                ybuf[c, 128 + 8 * g:128 + 8 * g + 8, 128 * t:128 * t + 128] = _val(outs[c][1])
        U = _dot(ZB.ld((0,), r, 128), M0.ld((0,), 0, 128))
        o = _rfft16([U[8 * a:8 * a + 8, :] for a in range(16)])

        def st(c, T, Tp):
            ybuf[c, 8 * g:8 * g + 8, 256:384] = _val(T)
            ybuf[c, 128 + 8 * g:128 + 8 * g + 8, 256:384] = _val(Tp)

        for c in (0, 8):
            Rc = o[c][0]
            st(c, Rc, (rollsg8(Rc[0]), Rc[1]))
        for c in range(1, 8):
            Rc, Ic = o[c]
            rt = (rollsg8(Rc[0]), Rc[1])
            it = (rollsg8(Ic[0]), Ic[1])
            st(c, _sub(Rc, it), _add(rt, Ic))
            st(16 - c, _add(Rc, it), _sub(rt, Ic))

    def wprep(h, ms):
        wv = (wr_v, wi_v)[h].bitcast(u32)
        lastv = (wrl_v, wil_v)[h]
        sub0 = lax.broadcasted_iota(jnp.int32, (8, 128), 0) == 0
        LO, HI = jnp.uint32(0xFFFF), jnp.uint32(0xFFFF0000)
        for m in ms:
            a = {k: [] for k in range(5)}
            for ig in range(4):
                v = [wv[m, pl.ds(r0 + 40 * ig, 8, stride=5), :] for r0 in range(5)]
                a[1].append((v[0] >> 16) | (v[3] << 16))
                a[4].append((v[2] & LO) | (v[4] & HI))
                a[2].append((v[1] & LO) | (v[3] & HI))
                a[3].append((v[1] >> 16) | (v[4] << 16))
                a[0].append((v[0] & LO) | (v[2] & HI))
            r320 = pltpu.bitcast(jnp.broadcast_to(lastv[:, 128 * m:128 * m + 128].astype(f32), (8, 128)), u32) >> 16
            a[0][0] = jnp.where(sub0, (a[0][0] & HI) | r320, a[0][0])
            T = pltpu.bitcast(_cat0(a[1] + a[4] + a[2] + a[3] + a[0] + a[0]), bf16)
            O = lax.dot_general(P1.ld((), 0, 128), T, NT, preferred_element_type=f32)
            for c in range(16):
                wc[c, 128 * h + 8 * m:128 * h + 8 * m + 8, :] = O[8 * c:8 * c + 8, :]

    def sfwd(c):
        Yr, Yi = ybuf[c, 0:128, :], ybuf[c, 128:256, :]
        k1 = _dot(CS.ld((c,), 0, 128), (Yr + Yi).astype(bf16))
        k2 = _dot(CS.ld((c,), 128, 128), Yi.astype(bf16))
        k3 = _dot(CS.ld((c,), 256, 128), Yr[:, 0:256].astype(bf16))
        Xr = k1 - k2
        Xi = _cat1([k1[:, 0:256] - k3, pltpu.roll(Xr[:, 256:384], 64, 1) * sF128])
        Wr, Wi = wc[c, 0:128, :], wc[c, 128:256, :]
        Zr, Zi = Xr * Wr - Xi * Wi, Xr * Wi + Xi * Wr
        return _cat0([Zr + Zi, Zi, Zr]).astype(bf16)

    def sinv(c, Z, first):
        if first:
            k1 = lax.dot_general(CS.ld((c,), 0, 128), Z[0:128], TN, preferred_element_type=f32)
            k2 = lax.dot_general(CS.ld((c,), 256, 128), Z[128:256], TN, preferred_element_type=f32)
            k3 = lax.dot_general(CS.ld((c,), 128, 128), Z[256:384, 0:256], TN, preferred_element_type=f32)
        else:
            k1 = _dot(CT.ld((c,), 0, 128), Z[0:128])
            k2 = _dot(CT.ld((c,), 128, 128), Z[128:256])
            k3 = _dot(CT.ld((c,), 256, 128), Z[256:384, 0:256])
        bbuf[c, 0:128, :] = k1 - k2
        bbuf[c, 128:256, 0:256] = k1[:, 0:256] - k3

    def sphase(first):
        order = [0, 4, 1, 5, 2, 6, 3, 7, 8, 12, 9, 13, 10, 14, 11, 15]
        if first:
            wait(cp_cs0)
        Z = sfwd(order[0])
        for i in range(15):
            if first and i == 7:
                wait(cp_cs1)
            Zn = sfwd(order[i + 1])
            sinv(order[i], Z, first)
            Z = Zn
        sinv(order[15], Z, first)

    def T1(g):
        for t in range(2):
            ins = [(bbuf[c, 8 * g:8 * g + 8, 128 * t:128 * (t + 1)],
                    bbuf[c, 128 + 8 * g:128 + 8 * g + 8, 128 * t:128 * (t + 1)]) for c in range(16)]
            outs = _fft16(ins, +1)
            for a in range(0, 16, 2):
                r = 128 * g + 8 * a
                ar = _cat0([_val(outs[a][0]), _val(outs[a + 1][0])])
                ai = _cat0([_val(outs[a][1]) * sF8, _val(outs[a + 1][1]) * sF8])
                AB.st((2 * t,), r, ar)
                AB.st((2 * t + 1,), r, ai)
                AB.st((5 + t,), r, ar + ai)
        Bv = [_pos(bbuf[c, 8 * g:8 * g + 8, 256:384]) for c in range(16)]
        P = {c: _add(Bv[c], Bv[16 - c]) for c in range(1, 8)}
        Q = {c: _pos(rollsg8(_val(_sub(Bv[c], Bv[16 - c])))) for c in range(1, 8)}
        outs = _irfft16(Bv[0], Bv[8], P, Q)
        for a in range(0, 16, 2):
            AB.st((4,), 128 * g + 8 * a, _cat0([_val(outs[a]), _val(outs[a + 1])]))

    def T2d(g):
        r0 = 128 * g
        TT = []
        for t in range(2):
            k1 = _dot(AB.ld((5 + t,), r0, 128), NI.ld((3 * t,), 0, 128))
            k2 = _dot(AB.ld((2 * t + 1,), r0, 128), NI.ld((3 * t + 1,), 0, 128))
            k3 = _dot(AB.ld((2 * t,), r0, 128), NI.ld((3 * t + 2,), 0, 128))
            TT.append(_cat1([k1 - k2, k1 + k3]))
        T0 = _dot(AB.ld((4,), r0, 128), M0.ld((1,), 0, 128))
        return TT[0], TT[1], T0

    def T2p(g, T):
        TA, TB, T0 = T
        r0 = 128 * g
        for lo in range(0, 128, 16):
            hi = lo + 16
            t0, t1r, t1i, t2r, t2i = T0[lo:hi], TA[lo:hi, 0:128], TA[lo:hi, 128:256], TB[lo:hi, 0:128], TB[lo:hi, 128:256]
            u, v = t1r + t2r, t1r - t2r
            mm, nn = t0 - 0.25 * u, K5 * v
            E1, E2 = mm + nn, mm - nn
            O1 = S51 * t1i + (S51 * K21) * t2i
            O2 = (S51 * K21) * t1i - S51 * t2i
            x = xs[r0 + lo:r0 + hi, :]
            x1 = [x[:, 0:128] + (t0 + u), x[:, 128:256] + (E1 - O1), x[:, 256:384] + (E2 - O2),
                  x[:, 384:512] + (E2 + O2), x[:, 512:640] + (E1 + O1)]
            xs[r0 + lo:r0 + hi, :] = _cat1(x1)
            m, r = stats(x1[0] + x1[1] + x1[2] + x1[3] + x1[4],
                         x1[0] * x1[0] + x1[1] * x1[1] + x1[2] * x1[2] + x1[3] * x1[3] + x1[4] * x1[4])
            xc = [xx - m for xx in x1]
            for p in range(5):
                XN.st((p,), r0 + lo, xc[p] * r)

    def M1(g):
        xn = _cat1([XN.ld((p,), 128 * g, 128) for p in range(5)])
        h = lax.dot_general(xn, _cat1([W1.ld((p,), 0, FM) for p in range(5)]), NT, preferred_element_type=f32)
        gm = _gelu2(h + b1_v[0:FM].astype(f32).reshape(1, FM)).astype(bf16)
        hT = lax.dot_general(_cat1([W1.ld((p,), FM, F - FM) for p in range(5)]), xn, NT, preferred_element_type=f32)
        gT = _gelu2(hT + b1col[...][:, 0:1])
        one = jnp.where(lax.broadcasted_iota(jnp.int32, (128, FP - F), 1) == 0, 1.0, 0.0).astype(f32)
        return _cat1([gm, _cat1([gT.T, one]).astype(bf16)])

    def M2(g, G, p0, p1, final):
        r = 128 * g
        for p in range(p0, p1):
            cols = slice(128 * p, 128 * p + 128)
            x2 = xs[r:r + 128, cols] + 0.5 * _dot(G, W2.ld((p,), 0, FP))
            if not final:
                xs[r:r + 128, cols] = x2
                continue
            for a in range(16):
                ost[a, 8 * g:8 * g + 8, cols] = x2[8 * a:8 * a + 8, :].astype(bf16)
            if g == NMINI - 1:
                pltpu.make_async_copy(ost.at[:, 8 * g:8 * g + 8, cols], o_hbm.at[:, 8 * g:8 * g + 8, cols],
                                      osem.at[g + p]).start()
            elif p == 4:
                pltpu.make_async_copy(ost.at[:, 8 * g:8 * g + 8], o_hbm.at[:, 8 * g:8 * g + 8], osem.at[g]).start()

    for i in range(len(XPIECES)):
        wait(cp_x[i])
        if i == 0:
            wait(cp_mf, cp_m0)
        gs = range(xp0[i], xp0[i] + XPIECES[i])
        for g in gs:
            xs[128 * g:128 * g + 128, :] = xst[:, 8 * g:8 * g + 8, :].astype(f32).reshape(128, D)
        for g in gs:
            H1(g)
        for g in gs:
            H2(g)
    wait(cp_p1, cp_wra, cp_wia)
    wprep(0, lo_m)
    wprep(1, lo_m)
    wait(cp_wrb)
    wprep(0, hi_m)
    wait(cp_wib)
    wprep(1, hi_m)
    sphase(True)
    wait(cp_ni)

    for layer in range(2):
        final = layer == 1
        T1(0)
        T2p(0, T2d(0))
        for g in range(NMINI):
            if not final and g > 0:
                H1(g - 1)
            if g + 1 < NMINI:
                T1(g + 1)
            if layer == 0 and g == 0:
                wait(cp_w1)
                bl = b1_v[FM:F].astype(f32).reshape(1, F - FM)
                b1col[...] = jnp.broadcast_to(bl.reshape(F - FM, 1), (F - FM, 128))
            G = M1(g)
            if not final and g > 0:
                H2(g - 1)
            if layer == 0 and g == 0:
                wait(cp_w2)
                row0 = lax.broadcasted_iota(jnp.int32, (FP - F, 128), 0) == 0
                b2r = 2.0 * b2_v[...].astype(f32).reshape(1, D)
                for p in range(5):
                    w2_v[p, F:FP, :] = jnp.where(
                        row0, jnp.broadcast_to(b2r[:, 128 * p:128 * p + 128], (FP - F, 128)), 0.0).astype(bf16)
            M2(g, G, 0, 1, final)
            if g + 1 < NMINI:
                T = T2d(g + 1)
            M2(g, G, 1, 5, final)
            if g + 1 < NMINI:
                T2p(g + 1, T)
        if not final:
            H1(NMINI - 1)
            H2(NMINI - 1)
            wait(cp_cst)
            sphase(False)
            wait(cp_sync)

    for g in range(NMINI - 1):
        pltpu.make_async_copy(ost.at[:, 8 * g:8 * g + 8], o_hbm.at[:, 8 * g:8 * g + 8], osem.at[g]).wait()
    g = NMINI - 1
    for p in range(5):
        cols = slice(128 * p, 128 * p + 128)
        pltpu.make_async_copy(ost.at[:, 8 * g:8 * g + 8, cols], o_hbm.at[:, 8 * g:8 * g + 8, cols],
                              osem.at[g + p]).wait()


@jax.jit
def pallas_interleave_layers__spectral_gfnet__dense_activation_gelu__prompt_kernel(
    A_x: jax.Array,
    A_w_r: jax.Array,
    A_w_i: jax.Array,
    B_x: jax.Array,
    B_w1: jax.Array,
    B_b1: jax.Array,
    B_w2: jax.Array,
    B_b2: jax.Array,
):
    del B_x
    hbm = pl.BlockSpec(memory_space=pltpu.HBM)
    V = pltpu.VMEM
    scratch = [
        V((16, 128, D), bf16), V((16, 320, 128), bf16), V((16, 320, 128), bf16), V((1, S), bf16), V((1, S), bf16),
        V((5, F, 128), bf16), V((F,), bf16), V((5, FP, 128), bf16), V((D,), bf16),
        V((6, 128, 128), bf16), V((6, 128, 128), bf16), V((2, 128, 128), bf16),
        V((16, 384, 128), bf16), V((16, 384, 128), bf16), V((128, 128), bf16),
        V((S, D), f32), V((16, 256, 384), f32), V((16, 256, 384), f32), V((16, 256, 384), f32),
        V((7, S, 128), bf16), V((7, S, 128), bf16), V((5, S, 128), bf16),
        V((16, 128, D), bf16), V((128, 128), bf16), V((F - FM, 128), f32),
        pltpu.SemaphoreType.DMA((72,)), pltpu.SemaphoreType.DMA((NMINI + 4,)),
    ]
    out = pl.pallas_call(
        _kernel,
        out_shape=jax.ShapeDtypeStruct((16, 128, D), bf16),
        in_specs=[hbm] * 13,
        out_specs=hbm,
        scratch_shapes=scratch,
        compiler_params=pltpu.CompilerParams(vmem_limit_bytes=110 * 1024 * 1024),
    )(A_x.reshape(16, 128, D), A_w_r.T, A_w_i.T, B_w1.T, B_b1, B_w2, B_b2,
      _K["MF"], _K["NI"], _K["M0"], _K["CSF"], _K["CST"], _K["P1"])
    return out.reshape(1, S, D)
```

```python
import numpy as np
import jax
import jax.numpy as jnp
from jax import lax
from jax.experimental import pallas as pl
from jax.experimental.pallas import tpu as pltpu
import ml_dtypes

S, D, F = 2048, 640, 1728
NMINI = 16
XPIECES = (1, 3, 4, 4, 4)
S51 = float(np.sin(2 * np.pi / 5))
K5 = float((np.cos(2 * np.pi / 5) - np.cos(4 * np.pi / 5)) / 2)
K21 = float(np.sin(4 * np.pi / 5) / np.sin(2 * np.pi / 5))


def _consts():
    e = np.arange(128)
    q = np.arange(128)
    sgn = np.where(e < 64, 1.0, -1.0)
    lA = np.where(e < 64, 1 + 5 * e, 4 + 5 * (e - 64))
    lB = np.where(e < 64, 2 + 5 * e, 3 + 5 * (e - 64))

    def three_mult(l):
        ph = 2 * np.pi * ((q[:, None] * l[None, :]) % D) / D
        c, s = np.cos(ph), sgn[None, :] * np.sin(ph)
        fwd = np.stack([c, -S51 * (c - s), c + s])
        inv = 2.0 / (S * D) * np.stack([c.T, (c + s).T, (s - c).T])
        return fwd, inv

    fA, iA = three_mult(lA)
    fB, iB = three_mult(lB)
    e0 = np.arange(64)
    l0 = np.where(e0 == 0, D // 2, 5 * e0)
    ph = 2 * np.pi * ((q[:, None] * l0[None, :]) % D) / D
    c, s = np.cos(ph), np.sin(ph)
    s = np.where(np.abs(s) < 1e-9, 0.0, s)
    cl = np.where(e0 == 0, 1.0, 2.0) / (S * D)
    M0 = np.concatenate([c, -s], axis=1)
    N0 = np.concatenate([c.T * cl[:, None], -s.T * cl[:, None]], axis=0)
    d = np.arange(128)
    CSF = np.zeros((16, 384, 128))
    CST = np.zeros((16, 384, 128))
    for cc in range(16):
        ph = 2 * np.pi * ((d[None, :] * (cc + 16 * d[:, None])) % S) / S
        C, Sn = np.cos(ph), np.sin(ph)
        CSF[cc] = np.concatenate([C, C - Sn, C + Sn], axis=0)
        CST[cc] = np.concatenate([C.T, C.T + Sn.T, C.T - Sn.T], axis=0)
    P1 = np.zeros((128, 128))
    for cc in range(16):
        for j in range(8):
            P1[8 * cc + j, 16 * j + cc] = 1.0
    out = dict(MF=np.concatenate([fA, fB]), NI=np.concatenate([iA, iB]), M0=np.stack([M0, N0]),
               CSF=CSF, CST=CST, P1=P1)
    return {k: v.astype(np.float32).astype(ml_dtypes.bfloat16) for k, v in out.items()}


_K = _consts()


def _add(a, b):
    if a[1] == b[1]:
        return (a[0] + b[0], a[1])
    if a[1] > 0:
        return (a[0] - b[0], 1)
    return (b[0] - a[0], 1)


def _neg(a):
    return (a[0], -a[1])


def _sub(a, b):
    return _add(a, _neg(b))


def _mulc(a, c):
    return (a[0] * float(c * a[1]), 1)


def _val(a):
    return a[0] if a[1] > 0 else -a[0]


def _pos(x):
    return (x, 1)


C16 = [float(np.cos(2 * np.pi * k / 16)) for k in range(16)]
S16 = [float(np.sin(2 * np.pi * k / 16)) for k in range(16)]
RH = float(np.sqrt(0.5))


def _tw(re, im, k, sign):
    k = k % 16
    kk = k if sign > 0 else (16 - k) % 16
    if kk == 0:
        return re, im
    if kk == 4:
        return _neg(im), re
    if kk == 8:
        return _neg(re), _neg(im)
    if kk == 12:
        return im, _neg(re)
    if kk == 2:
        return _mulc(_sub(re, im), RH), _mulc(_add(re, im), RH)
    if kk == 6:
        return _mulc(_add(re, im), -RH), _mulc(_sub(re, im), RH)
    if kk == 10:
        return _mulc(_sub(im, re), RH), _mulc(_add(re, im), -RH)
    if kk == 14:
        return _mulc(_add(re, im), RH), _mulc(_sub(im, re), RH)
    c, s = C16[kk], S16[kk]
    return _sub(_mulc(re, c), _mulc(im, s)), _add(_mulc(re, s), _mulc(im, c))


def _dft4(x, sign):
    (a_r, a_i), (b_r, b_i), (c_r, c_i), (d_r, d_i) = x
    s0r, s0i = _add(a_r, c_r), _add(a_i, c_i)
    s1r, s1i = _sub(a_r, c_r), _sub(a_i, c_i)
    s2r, s2i = _add(b_r, d_r), _add(b_i, d_i)
    s3r, s3i = _sub(b_r, d_r), _sub(b_i, d_i)
    X0 = (_add(s0r, s2r), _add(s0i, s2i))
    X2 = (_sub(s0r, s2r), _sub(s0i, s2i))
    if sign < 0:
        X1 = (_add(s1r, s3i), _sub(s1i, s3r))
        X3 = (_sub(s1r, s3i), _add(s1i, s3r))
    else:
        X1 = (_sub(s1r, s3i), _add(s1i, s3r))
        X3 = (_add(s1r, s3i), _sub(s1i, s3r))
    return [X0, X1, X2, X3]


def _fft16(x, sign):
    x = [(_pos(r), _pos(i)) for r, i in x]
    inner = []
    for n1 in range(4):
        y = _dft4([x[n1 + 4 * n2] for n2 in range(4)], sign)
        inner.append([_tw(y[k2][0], y[k2][1], n1 * k2, sign) for k2 in range(4)])
    out = [None] * 16
    for k2 in range(4):
        z = _dft4([inner[n1][k2] for n1 in range(4)], sign)
        for k1 in range(4):
            out[k2 + 4 * k1] = z[k1]
    return out


def _rfft16(x):
    x = [_pos(v) for v in x]
    y0, y2, y1 = [], [], []
    for n1 in range(4):
        a, b, c, d = x[n1], x[n1 + 4], x[n1 + 8], x[n1 + 12]
        s0, s1, s2, s3 = _add(a, c), _sub(a, c), _add(b, d), _sub(b, d)
        y0.append(_add(s0, s2))
        y2.append(_sub(s0, s2))
        y1.append((s1, _neg(s3)))
    out = {}
    a, b, c, d = y0
    s0, s1, s2, s3 = _add(a, c), _sub(a, c), _add(b, d), _sub(b, d)
    out[0] = (_add(s0, s2), None)
    out[8] = (_sub(s0, s2), None)
    out[4] = (s1, _neg(s3))
    u0, u1, u2, u3 = y2
    p = _mulc(_sub(u1, u3), RH)
    qv = _mulc(_add(u1, u3), RH)
    out[2] = (_add(u0, p), _neg(_add(u2, qv)))
    out[6] = (_sub(u0, p), _sub(u2, qv))
    t = [_tw(y1[n][0], y1[n][1], n, -1) for n in range(4)]
    z = _dft4(t, -1)
    out[1] = z[0]
    out[5] = z[1]
    out[7] = (z[2][0], _neg(z[2][1]))
    out[3] = (z[3][0], _neg(z[3][1]))
    return out


def _irfft16(B0, B8, P, Q):
    out = [None] * 16
    s, dlt = _add(B0, B8), _sub(B0, B8)
    f0 = [_add(s, P[4]), _sub(dlt, Q[4]), _sub(s, P[4]), _add(dlt, Q[4])]
    m, n = _sub(P[2], P[6]), _add(Q[2], Q[6])
    g = [_add(P[2], P[6]), _mulc(_sub(m, n), RH), _sub(Q[6], Q[2]), _mulc(_add(m, n), -RH)]
    V = [(P[1], Q[1]), (P[5], Q[5]), (P[7], _neg(Q[7])), (P[3], _neg(Q[3]))]
    U = _dft4(V, +1)
    for a in range(8):
        ur, ui = U[a % 4]
        if a == 0:
            h = ur
        elif a == 4:
            h = _neg(ui)
        else:
            h = _sub(_mulc(ur, C16[a]), _mulc(ui, S16[a]))
        base = _add(f0[a % 4], g[a % 4]) if a < 4 else _sub(f0[a % 4], g[a % 4])
        out[a] = _add(base, h)
        out[a + 8] = _sub(base, h)
    return out


def _gelu2(h):
    c0 = 0.7978845608028654
    u = h * (c0 + (c0 * 0.044715) * (h * h))
    return h * (1.0 + jnp.tanh(u))


f32, bf16, u32 = jnp.float32, jnp.bfloat16, jnp.uint32
NT = (((1,), (1,)), ((), ()))
TN = (((0,), (0,)), ((), ()))
FM = 128 * (F // 128)
FP = FM + 128


def _dot(a, b):
    return jnp.dot(a, b, preferred_element_type=f32)


def _cat1(parts):
    return jnp.concatenate(parts, axis=1)


def _cat0(parts):
    return jnp.concatenate(parts, axis=0)


class _B16:
    def __init__(self, raw):
        self.raw = raw
        self.words = raw.bitcast(u32)

    def ld(self, lead, r0, n):
        return pltpu.bitcast(self.words[(*lead, slice(r0 // 2, (r0 + n) // 2), slice(None))], bf16)

    def st(self, lead, r0, val):
        self.raw[(*lead, slice(r0, r0 + val.shape[0]), slice(None))] = val.astype(bf16)


def _kernel(x_hbm, wr_hbm, wi_hbm, w1_hbm, b1_hbm, w2_hbm, b2_hbm,
            mf_hbm, ni_hbm, m0_hbm, csf_hbm, cst_hbm, p1_hbm,
            o_hbm,
            xst, wr_v, wi_v, wrl_v, wil_v, w1_v, b1_v, w2_v, b2_v,
            mf_v, ni_v, m0_v, csf_v, cst_v, p1_v,
            xs, ybuf, bbuf, wc, zbuf, abuf, xnbuf, ost, sync_v, b1col, sems, osem):
    W1, W2 = _B16(w1_v), _B16(w2_v)
    MF, NI, M0, CS, CT, P1 = _B16(mf_v), _B16(ni_v), _B16(m0_v), _B16(csf_v), _B16(cst_v), _B16(p1_v)
    ZB, AB, XN = _B16(zbuf), _B16(abuf), _B16(xnbuf)

    nsem = [0]

    def start(src, dst):
        cp = pltpu.make_async_copy(src, dst, sems.at[nsem[0]])
        nsem[0] += 1
        cp.start()
        return [cp]

    def wait(*groups):
        for grp in groups:
            for cp in grp:
                cp.wait()

    xp0 = [sum(XPIECES[:i]) for i in range(len(XPIECES))]

    def x_copy(i):
        lo, hi = 8 * xp0[i], 8 * (xp0[i] + XPIECES[i])
        return start(x_hbm.at[:, lo:hi], xst.at[:, lo:hi])

    def w_copy(src, dst, last, ms):
        cps = sum([start(src.at[0:320, 128 * m:128 * m + 128], dst.at[m]) for m in ms], [])
        return cps + (start(src.at[320:321, :], last) if ms[0] == 0 else [])

    cp_x = [x_copy(0)]
    cp_mf = start(mf_hbm, mf_v)
    cp_m0 = start(m0_hbm, m0_v)
    cp_x += [x_copy(i) for i in range(1, len(XPIECES))]
    cp_p1 = start(p1_hbm, p1_v)
    lo_m, hi_m = list(range(0, 8)), list(range(8, 16))
    cp_wra = w_copy(wr_hbm, wr_v, wrl_v, lo_m)
    cp_wia = w_copy(wi_hbm, wi_v, wil_v, lo_m)
    cp_wrb = w_copy(wr_hbm, wr_v, wrl_v, hi_m)
    cp_wib = w_copy(wi_hbm, wi_v, wil_v, hi_m)
    cp_cs0 = start(csf_hbm.at[0:8], csf_v.at[0:8])
    cp_cs1 = start(csf_hbm.at[8:16], csf_v.at[8:16])
    cp_ni = start(ni_hbm, ni_v)
    cp_w1 = sum([start(w1_hbm.at[:, 128 * p:128 * p + 128], w1_v.at[p]) for p in range(5)], []) + start(b1_hbm, b1_v)
    cp_w2 = sum([start(w2_hbm.at[:, 128 * p:128 * p + 128], w2_v.at[p, 0:F]) for p in range(5)], []) + start(b2_hbm, b2_v)
    cp_cst = start(cst_hbm, cst_v)
    cp_sync = start(p1_hbm, sync_v)

    lane8 = lax.broadcasted_iota(jnp.int32, (8, 128), 1)
    sF8 = jnp.where(lane8 < 64, 1.0, -1.0).astype(f32)
    lane128 = lax.broadcasted_iota(jnp.int32, (128, 128), 1)
    sF128 = jnp.where(lane128 < 64, 1.0, -1.0).astype(f32)

    def rollsg8(v):
        return pltpu.roll(v, 64, 1) * sF8

    def stats(s1, s2):
        m = jnp.sum(s1, axis=-1, keepdims=True) * (1.0 / D)
        ex2 = jnp.sum(s2, axis=-1, keepdims=True) * (1.0 / D)
        return m, lax.rsqrt(jnp.maximum(ex2 - m * m, 0.0) + 1e-5)

    def H1(g):
        for r0 in range(128 * g, 128 * g + 128, 16):
            x = xs[r0:r0 + 16, :]
            x0, x1, x2, x3, x4 = [x[:, 128 * p:128 * (p + 1)] for p in range(5)]
            t1, t2, t3, t4 = x1 + x4, x2 + x3, x1 - x4, x2 - x3
            u, v = t1 + t2, t1 - t2
            z0 = x0 + u
            m, r = stats(z0, x0 * x0 + x1 * x1 + x2 * x2 + x3 * x3 + x4 * x4)
            z0 = z0 - 5.0 * m
            mm = x0 - 0.25 * u
            nn = K5 * v
            zs = [z * r for z in (z0, mm + nn, t3 + K21 * t4, mm - nn, K21 * t3 - t4)]
            for p in range(5):
                ZB.st((p,), r0, zs[p])
            ZB.st((5,), r0, zs[1] - S51 * zs[2])
            ZB.st((6,), r0, zs[3] - S51 * zs[4])

    def H2(g):
        r = 128 * g
        for t in range(2):
            k1 = _dot(ZB.ld((5 + t,), r, 128), MF.ld((3 * t,), 0, 128))
            k2 = _dot(ZB.ld((2 + 2 * t,), r, 128), MF.ld((3 * t + 1,), 0, 128))
            k3 = _dot(ZB.ld((1 + 2 * t,), r, 128), MF.ld((3 * t + 2,), 0, 128))
            Ur, Ui = k1 - k2, (k1 - k3) * sF128
            outs = _fft16([(Ur[8 * a:8 * a + 8], Ui[8 * a:8 * a + 8]) for a in range(16)], -1)
            for c in range(16):
                ybuf[c, 8 * g:8 * g + 8, 128 * t:128 * t + 128] = _val(outs[c][0])
                ybuf[c, 128 + 8 * g:128 + 8 * g + 8, 128 * t:128 * t + 128] = _val(outs[c][1])
        U = _dot(ZB.ld((0,), r, 128), M0.ld((0,), 0, 128))
        o = _rfft16([U[8 * a:8 * a + 8, :] for a in range(16)])

        def st(c, T, Tp):
            ybuf[c, 8 * g:8 * g + 8, 256:384] = _val(T)
            ybuf[c, 128 + 8 * g:128 + 8 * g + 8, 256:384] = _val(Tp)

        for c in (0, 8):
            Rc = o[c][0]
            st(c, Rc, (rollsg8(Rc[0]), Rc[1]))
        for c in range(1, 8):
            Rc, Ic = o[c]
            rt = (rollsg8(Rc[0]), Rc[1])
            it = (rollsg8(Ic[0]), Ic[1])
            st(c, _sub(Rc, it), _add(rt, Ic))
            st(16 - c, _add(Rc, it), _sub(rt, Ic))

    def wprep(h, ms):
        wv = (wr_v, wi_v)[h].bitcast(u32)
        lastv = (wrl_v, wil_v)[h]
        sub0 = lax.broadcasted_iota(jnp.int32, (8, 128), 0) == 0
        LO, HI = jnp.uint32(0xFFFF), jnp.uint32(0xFFFF0000)
        for m in ms:
            a = {k: [] for k in range(5)}
            for ig in range(4):
                v = [wv[m, pl.ds(r0 + 40 * ig, 8, stride=5), :] for r0 in range(5)]
                a[1].append((v[0] >> 16) | (v[3] << 16))
                a[4].append((v[2] & LO) | (v[4] & HI))
                a[2].append((v[1] & LO) | (v[3] & HI))
                a[3].append((v[1] >> 16) | (v[4] << 16))
                a[0].append((v[0] & LO) | (v[2] & HI))
            r320 = pltpu.bitcast(jnp.broadcast_to(lastv[:, 128 * m:128 * m + 128].astype(f32), (8, 128)), u32) >> 16
            a[0][0] = jnp.where(sub0, (a[0][0] & HI) | r320, a[0][0])
            T = pltpu.bitcast(_cat0(a[1] + a[4] + a[2] + a[3] + a[0] + a[0]), bf16)
            O = lax.dot_general(P1.ld((), 0, 128), T, NT, preferred_element_type=f32)
            for c in range(16):
                wc[c, 128 * h + 8 * m:128 * h + 8 * m + 8, :] = O[8 * c:8 * c + 8, :]

    def sfwd(c):
        Yr, Yi = ybuf[c, 0:128, :], ybuf[c, 128:256, :]
        k1 = _dot(CS.ld((c,), 0, 128), (Yr + Yi).astype(bf16))
        k2 = _dot(CS.ld((c,), 128, 128), Yi.astype(bf16))
        k3 = _dot(CS.ld((c,), 256, 128), Yr[:, 0:256].astype(bf16))
        Xr = k1 - k2
        Xi = _cat1([k1[:, 0:256] - k3, pltpu.roll(Xr[:, 256:384], 64, 1) * sF128])
        Wr, Wi = wc[c, 0:128, :], wc[c, 128:256, :]
        Zr, Zi = Xr * Wr - Xi * Wi, Xr * Wi + Xi * Wr
        return _cat0([Zr + Zi, Zi, Zr]).astype(bf16)

    def sinv(c, Z, first):
        if first:
            k1 = lax.dot_general(CS.ld((c,), 0, 128), Z[0:128], TN, preferred_element_type=f32)
            k2 = lax.dot_general(CS.ld((c,), 256, 128), Z[128:256], TN, preferred_element_type=f32)
            k3 = lax.dot_general(CS.ld((c,), 128, 128), Z[256:384, 0:256], TN, preferred_element_type=f32)
        else:
            k1 = _dot(CT.ld((c,), 0, 128), Z[0:128])
            k2 = _dot(CT.ld((c,), 128, 128), Z[128:256])
            k3 = _dot(CT.ld((c,), 256, 128), Z[256:384, 0:256])
        bbuf[c, 0:128, :] = k1 - k2
        bbuf[c, 128:256, 0:256] = k1[:, 0:256] - k3

    def sphase(first):
        order = [0, 4, 1, 5, 2, 6, 3, 7, 8, 12, 9, 13, 10, 14, 11, 15]
        if first:
            wait(cp_cs0)
        Z = sfwd(order[0])
        for i in range(15):
            if first and i == 7:
                wait(cp_cs1)
            Zn = sfwd(order[i + 1])
            sinv(order[i], Z, first)
            Z = Zn
        sinv(order[15], Z, first)

    def T1(g):
        for t in range(2):
            ins = [(bbuf[c, 8 * g:8 * g + 8, 128 * t:128 * (t + 1)],
                    bbuf[c, 128 + 8 * g:128 + 8 * g + 8, 128 * t:128 * (t + 1)]) for c in range(16)]
            outs = _fft16(ins, +1)
            for a in range(0, 16, 2):
                r = 128 * g + 8 * a
                ar = _cat0([_val(outs[a][0]), _val(outs[a + 1][0])])
                ai = _cat0([_val(outs[a][1]) * sF8, _val(outs[a + 1][1]) * sF8])
                AB.st((2 * t,), r, ar)
                AB.st((2 * t + 1,), r, ai)
                AB.st((5 + t,), r, ar + ai)
        Bv = [_pos(bbuf[c, 8 * g:8 * g + 8, 256:384]) for c in range(16)]
        P = {c: _add(Bv[c], Bv[16 - c]) for c in range(1, 8)}
        Q = {c: _pos(rollsg8(_val(_sub(Bv[c], Bv[16 - c])))) for c in range(1, 8)}
        outs = _irfft16(Bv[0], Bv[8], P, Q)
        for a in range(0, 16, 2):
            AB.st((4,), 128 * g + 8 * a, _cat0([_val(outs[a]), _val(outs[a + 1])]))

    def T2d(g):
        r0 = 128 * g
        TT = []
        for t in range(2):
            k1 = _dot(AB.ld((5 + t,), r0, 128), NI.ld((3 * t,), 0, 128))
            k2 = _dot(AB.ld((2 * t + 1,), r0, 128), NI.ld((3 * t + 1,), 0, 128))
            k3 = _dot(AB.ld((2 * t,), r0, 128), NI.ld((3 * t + 2,), 0, 128))
            TT.append(_cat1([k1 - k2, k1 + k3]))
        T0 = _dot(AB.ld((4,), r0, 128), M0.ld((1,), 0, 128))
        return TT[0], TT[1], T0

    def T2p(g, T):
        TA, TB, T0 = T
        r0 = 128 * g
        for lo in range(0, 128, 16):
            hi = lo + 16
            t0, t1r, t1i, t2r, t2i = T0[lo:hi], TA[lo:hi, 0:128], TA[lo:hi, 128:256], TB[lo:hi, 0:128], TB[lo:hi, 128:256]
            u, v = t1r + t2r, t1r - t2r
            mm, nn = t0 - 0.25 * u, K5 * v
            E1, E2 = mm + nn, mm - nn
            O1 = S51 * t1i + (S51 * K21) * t2i
            O2 = (S51 * K21) * t1i - S51 * t2i
            x = xs[r0 + lo:r0 + hi, :]
            x1 = [x[:, 0:128] + (t0 + u), x[:, 128:256] + (E1 - O1), x[:, 256:384] + (E2 - O2),
                  x[:, 384:512] + (E2 + O2), x[:, 512:640] + (E1 + O1)]
            xs[r0 + lo:r0 + hi, :] = _cat1(x1)
            m, r = stats(x1[0] + x1[1] + x1[2] + x1[3] + x1[4],
                         x1[0] * x1[0] + x1[1] * x1[1] + x1[2] * x1[2] + x1[3] * x1[3] + x1[4] * x1[4])
            xc = [xx - m for xx in x1]
            for p in range(5):
                XN.st((p,), r0 + lo, xc[p] * r)

    def M1(g):
        xn = _cat1([XN.ld((p,), 128 * g, 128) for p in range(5)])
        h = lax.dot_general(xn, _cat1([W1.ld((p,), 0, FM) for p in range(5)]), NT, preferred_element_type=f32)
        gm = _gelu2(h + b1_v[0:FM].astype(f32).reshape(1, FM)).astype(bf16)
        hT = lax.dot_general(_cat1([W1.ld((p,), FM, F - FM) for p in range(5)]), xn, NT, preferred_element_type=f32)
        gT = _gelu2(hT + b1col[...][:, 0:1])
        one = jnp.where(lax.broadcasted_iota(jnp.int32, (128, FP - F), 1) == 0, 1.0, 0.0).astype(f32)
        return _cat1([gm, _cat1([gT.T, one]).astype(bf16)])

    def M2(g, G, p0, p1, final):
        r = 128 * g
        for p in range(p0, p1):
            cols = slice(128 * p, 128 * p + 128)
            x2 = xs[r:r + 128, cols] + 0.5 * _dot(G, W2.ld((p,), 0, FP))
            if not final:
                xs[r:r + 128, cols] = x2
                continue
            for a in range(16):
                ost[a, 8 * g:8 * g + 8, cols] = x2[8 * a:8 * a + 8, :].astype(bf16)
            if g == NMINI - 1:
                pltpu.make_async_copy(ost.at[:, 8 * g:8 * g + 8, cols], o_hbm.at[:, 8 * g:8 * g + 8, cols],
                                      osem.at[g + p]).start()
            elif p == 4:
                pltpu.make_async_copy(ost.at[:, 8 * g:8 * g + 8], o_hbm.at[:, 8 * g:8 * g + 8], osem.at[g]).start()

    for i in range(len(XPIECES)):
        wait(cp_x[i])
        if i == 0:
            wait(cp_mf, cp_m0)
        gs = range(xp0[i], xp0[i] + XPIECES[i])
        for g in gs:
            xs[128 * g:128 * g + 128, :] = xst[:, 8 * g:8 * g + 8, :].astype(f32).reshape(128, D)
        for g in gs:
            H1(g)
        for g in gs:
            H2(g)
    wait(cp_p1, cp_wra, cp_wia)
    wprep(0, lo_m)
    wprep(1, lo_m)
    wait(cp_wrb)
    wprep(0, hi_m)
    wait(cp_wib)
    wprep(1, hi_m)
    sphase(True)
    wait(cp_ni, cp_w1)
    bl = b1_v[FM:F].astype(f32).reshape(1, F - FM)
    b1col[...] = jnp.broadcast_to(bl.reshape(F - FM, 1), (F - FM, 128))

    for layer in range(2):
        final = layer == 1
        T1(0)
        T2p(0, T2d(0))
        for g in range(NMINI):
            if not final and g > 0:
                H1(g - 1)
            G = M1(g)
            if not final and g > 0:
                H2(g - 1)
            if layer == 0 and g == 0:
                wait(cp_w2)
                row0 = lax.broadcasted_iota(jnp.int32, (FP - F, 128), 0) == 0
                b2r = 2.0 * b2_v[...].astype(f32).reshape(1, D)
                for p in range(5):
                    w2_v[p, F:FP, :] = jnp.where(
                        row0, jnp.broadcast_to(b2r[:, 128 * p:128 * p + 128], (FP - F, 128)), 0.0).astype(bf16)
            if g + 1 < NMINI:
                T1(g + 1)
            M2(g, G, 0, 1, final)
            if g + 1 < NMINI:
                T = T2d(g + 1)
            M2(g, G, 1, 5, final)
            if g + 1 < NMINI:
                T2p(g + 1, T)
        if not final:
            H1(NMINI - 1)
            H2(NMINI - 1)
            wait(cp_cst)
            sphase(False)
            wait(cp_sync)

    for g in range(NMINI - 1):
        pltpu.make_async_copy(ost.at[:, 8 * g:8 * g + 8], o_hbm.at[:, 8 * g:8 * g + 8], osem.at[g]).wait()
    g = NMINI - 1
    for p in range(5):
        cols = slice(128 * p, 128 * p + 128)
        pltpu.make_async_copy(ost.at[:, 8 * g:8 * g + 8, cols], o_hbm.at[:, 8 * g:8 * g + 8, cols],
                              osem.at[g + p]).wait()


@jax.jit
def pallas_interleave_layers__spectral_gfnet__dense_activation_gelu__prompt_kernel(
    A_x: jax.Array,
    A_w_r: jax.Array,
    A_w_i: jax.Array,
    B_x: jax.Array,
    B_w1: jax.Array,
    B_b1: jax.Array,
    B_w2: jax.Array,
    B_b2: jax.Array,
):
    del B_x
    hbm = pl.BlockSpec(memory_space=pltpu.HBM)
    V = pltpu.VMEM
    scratch = [
        V((16, 128, D), bf16), V((16, 320, 128), bf16), V((16, 320, 128), bf16), V((1, S), bf16), V((1, S), bf16),
        V((5, F, 128), bf16), V((F,), bf16), V((5, FP, 128), bf16), V((D,), bf16),
        V((6, 128, 128), bf16), V((6, 128, 128), bf16), V((2, 128, 128), bf16),
        V((16, 384, 128), bf16), V((16, 384, 128), bf16), V((128, 128), bf16),
        V((S, D), f32), V((16, 256, 384), f32), V((16, 256, 384), f32), V((16, 256, 384), f32),
        V((7, S, 128), bf16), V((7, S, 128), bf16), V((5, S, 128), bf16),
        V((16, 128, D), bf16), V((128, 128), bf16), V((F - FM, 128), f32),
        pltpu.SemaphoreType.DMA((72,)), pltpu.SemaphoreType.DMA((NMINI + 4,)),
    ]
    out = pl.pallas_call(
        _kernel,
        out_shape=jax.ShapeDtypeStruct((16, 128, D), bf16),
        in_specs=[hbm] * 13,
        out_specs=hbm,
        scratch_shapes=scratch,
        compiler_params=pltpu.CompilerParams(vmem_limit_bytes=110 * 1024 * 1024),
    )(A_x.reshape(16, 128, D), A_w_r.T, A_w_i.T, B_w1.T, B_b1, B_w2, B_b2,
      _K["MF"], _K["NI"], _K["M0"], _K["CSF"], _K["CST"], _K["P1"])
    return out.reshape(1, S, D)
```
